```python
import jax
import jax.numpy as jnp

def _softmax(x, axis=-1):
    return jax.nn.softmax(x, axis=axis)

def _gelu(x):
    return jax.nn.gelu(x, approximate=True)

def _silu(x):
    return jax.nn.silu(x)

def _sigmoid(x):
    return jax.nn.sigmoid(x)

def _layernorm(x, axis=-1, eps=1e-05):
    m = jnp.mean(x, axis=axis, keepdims=True)
    v = jnp.var(x, axis=axis, keepdims=True)
    return (x - m) / jnp.sqrt(v + eps)

def _scatter_add(tgt, idx, src, axis=0):
    return tgt.at[idx].add(src)

def _segment_sum(src, seg, n):
    return jax.ops.segment_sum(src, seg, n)

class _Rng:

    def __init__(self, key):
        self._k = key

    def _next(self):
        self._k, sub = jax.random.split(self._k)
        return sub

    def normal(self, shape):
        return jax.random.normal(self._next(), shape, dtype=jnp.bfloat16)

    def randint(self, lo, hi, shape):
        return jax.random.randint(self._next(), shape, lo, hi, dtype=jnp.int32)

    def uniform(self, shape, lo=0.0, hi=1.0):
        return jax.random.uniform(self._next(), shape, jnp.bfloat16, lo, hi)

    def permutation(self, n):
        return jax.random.permutation(self._next(), n)
kernel_name = 'interleave_layers__memory_aug_infini_attn__moe_arch_mod__prompt'

def setup_inputs():
    _rng = _Rng(jax.random.key(int.from_bytes(__import__("os").urandom(4), "little")))
    _w = lambda a: (lambda t: t.astype(jnp.bfloat16) if jnp.issubdtype(t.dtype, jnp.floating) else t)(jnp.asarray(a))

    def _A_setup():
        B, S, D, H = (1, 2048, 1024, 32)
        N = 4
        L = max(1, S // N)
        sc = D ** (-0.5)
        return {'x': _w((lambda *s: _rng.normal(s) * 0.05)(B, N * L, D)), 'wq': _w((lambda *s: _rng.normal(s) * 0.05)(D, D) * sc), 'wk': _w((lambda *s: _rng.normal(s) * 0.05)(D, D) * sc), 'wv': _w((lambda *s: _rng.normal(s) * 0.05)(D, D) * sc), 'wo': _w((lambda *s: _rng.normal(s) * 0.05)(D, D) * sc), 'beta': _w((lambda *s: _rng.normal(s) * 0.05)(H))}
    _A_in = _A_setup()

    def _B_setup():
        B, S, D, F, C = (1, 2048, 1024, 3584, 2)
        return {'x': _w((lambda *s: _rng.normal(s) * 0.05)(B, S, D)), 'w_r': _w((lambda *s: _rng.normal(s) * 0.05)(D)), 'w_gate': _w((lambda *s: _rng.normal(s) * 0.05)(D, F)), 'w_up': _w((lambda *s: _rng.normal(s) * 0.05)(D, F)), 'w_down': _w((lambda *s: _rng.normal(s) * 0.05)(F, D))}
    _B_in = _B_setup()
    return {'A_x': _A_in['x'], 'A_wq': _A_in['wq'], 'A_wk': _A_in['wk'], 'A_wv': _A_in['wv'], 'A_wo': _A_in['wo'], 'A_beta': _A_in['beta'], 'B_x': _B_in['x'], 'B_w_r': _B_in['w_r'], 'B_w_gate': _B_in['w_gate'], 'B_w_up': _B_in['w_up'], 'B_w_down': _B_in['w_down']}

def reference(A_x, A_wq, A_wk, A_wv, A_wo, A_beta, B_x, B_w_r, B_w_gate, B_w_up, B_w_down):

    def _A_ref(x, wq, wk, wv, wo, beta):
        B, S, D = x.shape
        H = 32
        Dh = D // H
        N = 4
        L = S // N
        q = (lambda x, *d: x.transpose(*d))((x @ wq).reshape(B, S, H, Dh), 0, 2, 1, 3).reshape(B, H, N, L, Dh)
        k = (lambda x, *d: x.transpose(*d))((x @ wk).reshape(B, S, H, Dh), 0, 2, 1, 3).reshape(B, H, N, L, Dh)
        v = (lambda x, *d: x.transpose(*d))((x @ wv).reshape(B, S, H, Dh), 0, 2, 1, 3).reshape(B, H, N, L, Dh)
        phi = lambda t: jnp.where(t > 0, t + 1.0, jnp.exp(t))
        scale = Dh ** (-0.5)
        ar = jnp.arange(L)
        mask = (lambda x, dt: x.astype(dt))(ar[:, None] < ar[None, :], x.dtype) * -1000000000.0
        g = _sigmoid(beta).reshape(1, H, 1, 1)
        M = jnp.einsum('bhd,bhe->bhde', q[:, :, 0, 0, :] * 0.0, q[:, :, 0, 0, :] * 0.0)
        z = q[:, :, 0, 0, :] * 0.0
        outs = []
        for s in range(N):
            qs, ks, vs = (q[:, :, s].copy(), k[:, :, s].copy(), v[:, :, s].copy())
            logits = jnp.einsum('bhqd,bhkd->bhqk', qs, ks) * scale + mask
            p = _softmax(logits, axis=-1)
            a_dot = jnp.einsum('bhqk,bhkd->bhqd', p, vs)
            pq = phi(qs)
            num = jnp.einsum('bhld,bhde->bhle', pq, M)
            den = jnp.einsum('bhld,bhd->bhl', pq, z)[..., None] + 1e-06
            a_mem = num / den
            o = g * a_mem + (1.0 - g) * a_dot
            outs.append(o)
            pk = phi(ks)
            M = M + jnp.einsum('bhld,bhle->bhde', pk, vs)
            z = z + jnp.einsum('bhld->bhd', pk)
        o = (lambda x, *d: x.transpose(*d))(jnp.stack(outs, 2).reshape(B, H, S, Dh), 0, 2, 1, 3).reshape(B, S, D)
        return o @ wo

    def _B_ref(x, w_r, w_gate, w_up, w_down):
        B, S, D = x.shape
        C = 2
        r = x @ w_r
        idx = jnp.argsort(-r, axis=-1)[:, :C]
        idx_e = jnp.repeat(idx.reshape(B, C, 1), D, axis=2)
        x_sel = jnp.take_along_axis(x, idx_e, axis=1)
        g = _silu(x_sel @ w_gate)
        u = x_sel @ w_up
        y = g * u @ w_down
        r_sel = _sigmoid(jnp.take_along_axis(r, idx, axis=1))
        y = y * r_sel.reshape(B, C, 1)
        b_off = (jnp.arange(B) * S).reshape(B, 1)
        flat_idx = (idx + b_off).reshape(B * C)
        zero = (x * 0.0).reshape(B * S, D)
        upd = _scatter_add(zero, flat_idx, y.reshape(B * C, D), axis=0)
        return x + upd.reshape(B, S, D)
    x = A_x
    x = x + _A_ref(_layernorm(x, axis=-1), A_wq, A_wk, A_wv, A_wo, A_beta)
    x = x + _B_ref(_layernorm(x, axis=-1), B_w_r, B_w_gate, B_w_up, B_w_down)
    x = x + _A_ref(_layernorm(x, axis=-1), A_wq, A_wk, A_wv, A_wo, A_beta)
    x = x + _B_ref(_layernorm(x, axis=-1), B_w_r, B_w_gate, B_w_up, B_w_down)
    return x
```

```python
import functools
import math

import jax
import jax.numpy as jnp
from jax import lax
import jax.experimental.pallas as pl
import jax.experimental.pallas.tpu as pltpu

S = 2048
D = 1024
H = 32
DH = 32
NSEG = 4
L = S // NSEG
F = 3584
G = 8
HG = 4
QB = 128
NQB = L // QB
MR = 144
EPS = 1e-5
LOG2E = math.log2(math.e)
QSCALE = (DH ** -0.5) * LOG2E
NEG = -1e9 * LOG2E

f32 = jnp.float32
bf16 = jnp.bfloat16

NT = (((1,), (1,)), ((), ()))


def _rbf(x):
    return x.astype(bf16).astype(f32)


def _ln(x):
    m = jnp.sum(x, axis=1, keepdims=True) * (1.0 / D)
    c = x - m
    v = jnp.sum(c * c, axis=1, keepdims=True) * (1.0 / D)
    sd = _rbf(jnp.sqrt(_rbf(_rbf(v) + EPS)))
    return (x - _rbf(m)) * (1.0 / sd)


def _phi(t):
    return jnp.where(t > 0, t + 1.0, jnp.exp(t))


def _sigmoid(t):
    return 1.0 / (1.0 + jnp.exp(-t))


def _dot(a, b):
    return jnp.dot(a, b, preferred_element_type=f32)


def _dot_nt(a, b):
    return lax.dot_general(a, b, NT, preferred_element_type=f32)


def _colsum(p):
    n = p.shape[0]
    parts = [p[j * 8:(j + 1) * 8] for j in range(n // 8)]
    while len(parts) > 1:
        nxt = [parts[j] + parts[j + 1] for j in range(0, len(parts) - 1, 2)]
        if len(parts) % 2:
            nxt.append(parts[-1])
        parts = nxt
    return jnp.sum(parts[0], axis=0, keepdims=True)


def _kernel(x_hbm, wq_hbm, wk_hbm, wv_hbm, wo_hbm, beta_ref, wr_ref, wg_hbm, wu_hbm, wd_hbm,
            out_hbm,
            X, XB, XN, WKQ, WV, WVT, WO, WG, WU, WD,
            KB, QS, PQ, PK, VT, OB, MEM, R, GATE, MASK, MMASK, WR,
            sem_x, sem_w, sem_f, sem_o):

    def x_copy(s):
        return pltpu.make_async_copy(x_hbm.at[0, pl.ds(s * L, L), :], X.at[pl.ds(s * L, L), :], sem_x.at[s])

    def wk_copy(g):
        return pltpu.make_async_copy(wk_hbm.at[:, pl.ds(g * 128, 128)], WKQ.at[g, :, pl.ds(0, 128)], sem_w.at[g])

    def wq_copy(g):
        return pltpu.make_async_copy(wq_hbm.at[:, pl.ds(g * 128, 128)], WKQ.at[g, :, pl.ds(128, 128)],
                                     sem_w.at[G + g])

    def wv_copy(g):
        return pltpu.make_async_copy(wv_hbm.at[:, pl.ds(g * 128, 128)], WV.at[g], sem_w.at[2 * G + g])

    wo_copy = pltpu.make_async_copy(wo_hbm, WO, sem_w.at[3 * G])
    wg_copy = pltpu.make_async_copy(wg_hbm, WG, sem_f.at[0])
    wu_copy = pltpu.make_async_copy(wu_hbm, WU, sem_f.at[1])
    wd_copy = pltpu.make_async_copy(wd_hbm, WD, sem_f.at[2])

    def out_copy(s):
        return pltpu.make_async_copy(X.at[pl.ds(s * L, L), :], out_hbm.at[0, pl.ds(s * L, L), :], sem_o.at[s])

    x_copy(0).start()
    for g in range(G):
        wv_copy(g).start()
        wk_copy(g).start()
        wq_copy(g).start()
    wo_copy.start()
    for s in range(1, NSEG):
        x_copy(s).start()
    wg_copy.start()
    wu_copy.start()
    wd_copy.start()

    row = lax.broadcasted_iota(jnp.int32, (128, 128), 0)
    col = lax.broadcasted_iota(jnp.int32, (128, 128), 1)
    MASK[...] = jnp.where(row > col, NEG, 0.0).astype(f32)
    r144 = lax.broadcasted_iota(jnp.int32, (MR, 128), 0)
    c144 = lax.broadcasted_iota(jnp.int32, (MR, 128), 1)
    head_of_row = jnp.where(r144 < 128, r144 >> 5, r144 - 128)
    MMASK[...] = jnp.where(head_of_row == (c144 >> 5), 1.0, 0.0).astype(f32)
    MEM[...] = jnp.zeros(MEM.shape, f32)
    VT[:, 128:MR, :] = jnp.ones((2, MR - 128, L), bf16)
    R[...] = jnp.full(R.shape, -jnp.inf, f32)
    gsig = _rbf(_sigmoid(beta_ref[...].astype(f32)))
    r32 = lax.broadcasted_iota(jnp.int32, (H, H), 0)
    c32 = lax.broadcasted_iota(jnp.int32, (H, H), 1)
    gcol = jnp.sum(jnp.where(r32 == c32, jnp.broadcast_to(gsig, (H, H)), 0.0), axis=1, keepdims=True)
    GATE[...] = jnp.broadcast_to(gcol, (H, 128))
    WR[...] = jnp.broadcast_to(wr_ref[...].astype(f32), (8, D))

    x_copy(0).wait()
    for c in range(L // 128):
        XN[c * 128:(c + 1) * 128, :] = _ln(X[c * 128:(c + 1) * 128, :].astype(f32)).astype(bf16)

    for g in range(G):
        wv_copy(g).wait()
        WVT[g] = WV[g].T
        wk_copy(g).wait()
        wq_copy(g).wait()
    wo_copy.wait()
    for s in range(1, NSEG):
        x_copy(s).wait()

    lane128 = lax.broadcasted_iota(jnp.int32, (QB // 2, 128), 1) >> 5

    def proj(g, slot):
        xn = XN[...]
        kq = _dot(xn, WKQ[g])
        k = kq[:, :128]
        q = kq[:, 128:]
        KB[slot] = k.astype(bf16)
        PK[slot] = _phi(k).astype(bf16)
        QS[slot] = (q * QSCALE).astype(bf16)
        PQ[slot] = _phi(q).astype(bf16)
        VT[slot, 0:128, :] = _dot_nt(WVT[g], xn).astype(bf16)

    def attn(g, slot, keep):
        mem = MEM[g]
        mrd = _dot_nt((mem * MMASK[...]).astype(bf16), PQ[slot])
        upd = _dot(VT[slot], PK[slot])
        MEM[g] = (mem + upd) * keep
        gates = [GATE[pl.ds(g * HG + h, 1), :] for h in range(HG)]
        for i in range(NQB - 1, -1, -1):
            n = QB * (i + 1)
            qi = pltpu.bitcast(QS[slot, i * QB:(i + 1) * QB, :], jnp.uint32)
            qm = jnp.concatenate(
                [pltpu.bitcast(jnp.where(lane128 == h, qi, jnp.uint32(0)), bf16) for h in range(HG)], axis=0)
            st = _dot_nt(KB[slot, 0:n, :], qm)
            outs = []
            for h in range(HG):
                sh = st[:, h * QB:(h + 1) * QB]
                sd = sh[n - QB:, :] + MASK[...]
                sh = sd if i == 0 else jnp.concatenate([sh[:n - QB, :], sd], axis=0)
                m = jnp.max(sh, axis=0, keepdims=True)
                p = jnp.exp2(sh - m)
                l = _colsum(p)
                o = _dot(VT[slot, h * DH:(h + 1) * DH, 0:n], p.astype(bf16))
                num = mrd[h * DH:(h + 1) * DH, i * QB:(i + 1) * QB]
                den = mrd[128 + h:129 + h, i * QB:(i + 1) * QB] + 1e-6
                gt = gates[h]
                outs.append(num * (gt / den) + o * ((1.0 - gt) / l))
            ot = jnp.concatenate(outs, axis=0)
            OB[g, i * QB:(i + 1) * QB, :] = ot.T.astype(bf16)

    def epilogue(s, s_next):
        base = pl.multiple_of(s * L, L)
        nbase = pl.multiple_of(s_next * L, L)
        rs = []
        for c in range(L // 128):
            rows = pl.ds(base + c * 128, 128)
            o = jnp.concatenate([OB[g, c * 128:(c + 1) * 128, :] for g in range(G)], axis=1)
            y = _dot(o, WO[...])
            x1 = _rbf(X[rows, :].astype(f32) + _rbf(y))
            xb16 = _ln(x1).astype(bf16)
            xb = xb16.astype(f32)
            XB[rows, :] = xb16
            X[rows, :] = (x1 + xb).astype(bf16)
            wr = WR[0:1, :]
            part = xb[:, 0:128] * wr[:, 0:128]
            for j in range(1, D // 128):
                part = part + xb[:, j * 128:(j + 1) * 128] * wr[:, j * 128:(j + 1) * 128]
            rs.append(_colsum(part.T))
        R[pl.ds(s, 1), :] = _rbf(jnp.concatenate(rs, axis=1))
        for c in range(L // 128):
            nrows = pl.ds(nbase + c * 128, 128)
            XN[c * 128:(c + 1) * 128, :] = _ln(X[nrows, :].astype(f32)).astype(bf16)

    def ffn():
        r = R[...]
        idx = (lax.broadcasted_iota(jnp.int32, (8, L), 0) * L + lax.broadcasted_iota(jnp.int32, (8, L), 1))
        m1 = jnp.max(r)
        i1 = jnp.min(jnp.where(r == m1, idx, S - 1))
        r2 = jnp.where(idx == i1, -jnp.inf, r)
        m2 = jnp.max(r2)
        i2 = jnp.min(jnp.where((r2 == m2) & (idx != i1), idx, S - 1))
        i1 = jnp.clip(i1, 0, S - 1)
        i2 = jnp.clip(i2, 0, S - 1)
        sub = lax.broadcasted_iota(jnp.int32, (16, D), 0)
        sel = []
        for ii in (i1, i2):
            b = pl.multiple_of((ii >> 4) << 4, 16)
            blk = XB[pl.ds(b, 16), :].astype(f32)
            sel.append(jnp.sum(jnp.where(sub == (ii & 15), blk, 0.0), axis=0, keepdims=True))
        xs = jnp.where(sub == 0, sel[0], jnp.where(sub == 1, sel[1], 0.0)).astype(bf16)
        gt = _rbf(_dot(xs, WG[...]))
        up = _rbf(_dot(xs, WU[...]))
        hh = (_rbf(gt * _sigmoid(gt)) * up).astype(bf16)
        y = _rbf(_dot(hh, WD[...]))
        for j, (ii, mm) in enumerate(((i1, m1), (i2, m2))):
            sg = _rbf(_sigmoid(jnp.full((1, D), mm, f32)))
            yj = _rbf(y[j:j + 1, :] * sg)
            b = pl.multiple_of((ii >> 4) << 4, 16)
            blk = X[pl.ds(b, 16), :].astype(f32)
            X[pl.ds(b, 16), :] = jnp.where(sub == (ii & 15), blk + yj, blk).astype(bf16)
        return i1, i2

    def step(t, carry):
        s = t % NSEG
        keep = jnp.where(s == NSEG - 1, 0.0, 1.0).astype(f32)
        proj(0, 0)

        def gbody(g, c):
            slot = g % 2
            attn(g, slot, keep)
            proj(g + 1, 1 - slot)
            return c

        lax.fori_loop(0, G - 1, gbody, 0)
        attn(G - 1, (G - 1) % 2, keep)
        epilogue(s, (s + 1) % NSEG)

        @pl.when(jnp.logical_and(t >= NSEG, s < NSEG - 1))
        def _():
            out_copy(s).start()

        @pl.when(t == NSEG - 1)
        def _():
            wg_copy.wait()
            wu_copy.wait()
            wd_copy.wait()
            i1, i2 = ffn()
            for ii in (i1, i2):
                @pl.when(ii < L)
                def _():
                    b = pl.multiple_of((ii >> 4) << 4, 16)
                    XN[pl.ds(b, 16), :] = _ln(X[pl.ds(b, 16), :].astype(f32)).astype(bf16)

        return carry

    lax.fori_loop(0, 2 * NSEG, step, 0)

    for s in range(NSEG - 1):
        out_copy(s).wait()
    i1, i2 = ffn()
    out_copy(NSEG - 1).start()
    out_copy(NSEG - 1).wait()
    for j, ii in enumerate((i1, i2)):
        b = pl.multiple_of((ii >> 4) << 4, 16)
        cp = pltpu.make_async_copy(X.at[pl.ds(b, 16), :], out_hbm.at[0, pl.ds(b, 16), :], sem_o.at[j])
        cp.start()
        cp.wait()


@jax.jit
def pallas_interleave_layers__memory_aug_infini_attn__moe_arch_mod__prompt_kernel(
    A_x: jax.Array,
    A_wq: jax.Array,
    A_wk: jax.Array,
    A_wv: jax.Array,
    A_wo: jax.Array,
    A_beta: jax.Array,
    B_x: jax.Array,
    B_w_r: jax.Array,
    B_w_gate: jax.Array,
    B_w_up: jax.Array,
    B_w_down: jax.Array,
):
    del B_x
    any_spec = pl.BlockSpec(memory_space=pl.ANY)
    vmem_spec = pl.BlockSpec(memory_space=pltpu.VMEM)
    scratch = [
        pltpu.VMEM((S, D), bf16),
        pltpu.VMEM((S, D), bf16),
        pltpu.VMEM((L, D), bf16),
        pltpu.VMEM((G, D, 256), bf16),
        pltpu.VMEM((G, D, 128), bf16),
        pltpu.VMEM((G, 128, D), bf16),
        pltpu.VMEM((D, D), bf16),
        pltpu.VMEM((D, F), bf16),
        pltpu.VMEM((D, F), bf16),
        pltpu.VMEM((F, D), bf16),
        pltpu.VMEM((2, L, 128), bf16),
        pltpu.VMEM((2, L, 128), bf16),
        pltpu.VMEM((2, L, 128), bf16),
        pltpu.VMEM((2, L, 128), bf16),
        pltpu.VMEM((2, MR, L), bf16),
        pltpu.VMEM((G, L, 128), bf16),
        pltpu.VMEM((G, MR, 128), f32),
        pltpu.VMEM((8, L), f32),
        pltpu.VMEM((H, 128), f32),
        pltpu.VMEM((128, 128), f32),
        pltpu.VMEM((MR, 128), f32),
        pltpu.VMEM((8, D), f32),
        pltpu.SemaphoreType.DMA((NSEG,)),
        pltpu.SemaphoreType.DMA((3 * G + 1,)),
        pltpu.SemaphoreType.DMA((3,)),
        pltpu.SemaphoreType.DMA((NSEG,)),
    ]
    return pl.pallas_call(
        _kernel,
        out_shape=jax.ShapeDtypeStruct((1, S, D), bf16),
        in_specs=[any_spec, any_spec, any_spec, any_spec, any_spec, vmem_spec, vmem_spec,
                  any_spec, any_spec, any_spec],
        out_specs=any_spec,
        scratch_shapes=scratch,
        compiler_params=pltpu.CompilerParams(vmem_limit_bytes=100 * 2 ** 20),
    )(A_x, A_wq, A_wk, A_wv, A_wo, A_beta.reshape(1, H), B_w_r.reshape(1, D), B_w_gate, B_w_up, B_w_down)
```

```python
import functools
import math

import jax
import jax.numpy as jnp
from jax import lax
import jax.experimental.pallas as pl
import jax.experimental.pallas.tpu as pltpu

S = 2048
D = 1024
H = 32
DH = 32
NSEG = 4
L = S // NSEG
F = 3584
G = 8
HG = 4
QB = 128
NQB = L // QB
MR = 144
CH = L // G
U = 2
EPS = 1e-5
LOG2E = math.log2(math.e)
QSCALE = (DH ** -0.5) * LOG2E
NEG = -1e9 * LOG2E
IMIN = -2 ** 31

f32 = jnp.float32
bf16 = jnp.bfloat16
i32 = jnp.int32

NT = (((1,), (1,)), ((), ()))


def _rbf(x):
    return x.astype(bf16).astype(f32)


def _ln(x):
    m = jnp.sum(x, axis=1, keepdims=True) * (1.0 / D)
    c = x - m
    v = jnp.sum(c * c, axis=1, keepdims=True) * (1.0 / D)
    sd = _rbf(jnp.sqrt(_rbf(_rbf(v) + EPS)))
    return (x - _rbf(m)) * (1.0 / sd)


def _phi(t):
    return jnp.where(t > 0, t + 1.0, jnp.exp(t))


def _sigmoid(t):
    return 1.0 / (1.0 + jnp.exp(-t))


def _dot(a, b):
    return jnp.dot(a, b, preferred_element_type=f32)


def _dot_nt(a, b):
    return lax.dot_general(a, b, NT, preferred_element_type=f32)


def _colsum(p):
    n = p.shape[0]
    parts = [p[j * 8:(j + 1) * 8] for j in range(n // 8)]
    while len(parts) > 1:
        nxt = [parts[j] + parts[j + 1] for j in range(0, len(parts) - 1, 2)]
        if len(parts) % 2:
            nxt.append(parts[-1])
        parts = nxt
    return jnp.sum(parts[0], axis=0, keepdims=True)


def _kernel(x_hbm, wq_hbm, wk_hbm, wv_hbm, wo_hbm, beta_ref, wr_ref, wg_hbm, wu_hbm, wd_hbm,
            out_hbm,
            X, XB, XN, W3, WO, WG, WU, WD,
            KB, QS, PQ, PK, VT, OB, MEM, TOP, GATE, MASK, MMASK, WR,
            sem_x, sem_w, sem_f, sem_o):

    def x0_copy(c):
        return pltpu.make_async_copy(x_hbm.at[0, pl.ds(c * 128, 128), :], X.at[pl.ds(c * 128, 128), :],
                                     sem_x.at[NSEG + c])

    def x_copy(s):
        return pltpu.make_async_copy(x_hbm.at[0, pl.ds(s * L, L), :], X.at[pl.ds(s * L, L), :], sem_x.at[s])

    def w_copies(g):
        col = pl.multiple_of(g * 128, 128)
        return [pltpu.make_async_copy(w.at[:, pl.ds(col, 128)], W3.at[g, :, pl.ds(j * 128, 128)],
                                      sem_w.at[3 * g + j])
                for j, w in enumerate((wk_hbm, wq_hbm, wv_hbm))]

    wo_copy = pltpu.make_async_copy(wo_hbm, WO, sem_w.at[3 * G])
    wg_copy = pltpu.make_async_copy(wg_hbm, WG, sem_f.at[0])
    wu_copy = pltpu.make_async_copy(wu_hbm, WU, sem_f.at[1])
    wd_copy = pltpu.make_async_copy(wd_hbm, WD, sem_f.at[2])

    def out_copy(s):
        base = pl.multiple_of(s * L, L)
        return pltpu.make_async_copy(X.at[pl.ds(base, L), :], out_hbm.at[0, pl.ds(base, L), :], sem_o.at[s])

    x0_copy(0).start()
    for cp in w_copies(0):
        cp.start()
    for c in range(1, 4):
        x0_copy(c).start()
    for g in range(1, 1 + U):
        for cp in w_copies(g):
            cp.start()
    x_copy(1).start()

    row = lax.broadcasted_iota(i32, (128, 128), 0)
    col = lax.broadcasted_iota(i32, (128, 128), 1)
    MASK[...] = jnp.where(row > col, NEG, 0.0).astype(f32)
    r144 = lax.broadcasted_iota(i32, (MR, 128), 0)
    c144 = lax.broadcasted_iota(i32, (MR, 128), 1)
    head_of_row = jnp.where(r144 < 128, r144 >> 5, r144 - 128)
    MMASK[...] = jnp.where(head_of_row == (c144 >> 5), 1.0, 0.0).astype(f32)
    VT[:, 128:MR, :] = jnp.ones((2 * G, MR - 128, L), bf16)
    gsig = _rbf(_sigmoid(beta_ref[...].astype(f32)))
    r32 = lax.broadcasted_iota(i32, (H, H), 0)
    c32 = lax.broadcasted_iota(i32, (H, H), 1)
    gcol = jnp.sum(jnp.where(r32 == c32, jnp.broadcast_to(gsig, (H, H)), 0.0), axis=1, keepdims=True)
    GATE[...] = jnp.broadcast_to(gcol, (H, 128))
    WR[...] = jnp.broadcast_to(wr_ref[...].astype(f32), (8, D))

    for c in range(L // 128):
        x0_copy(c).wait()
        XN[0, c * 128:(c + 1) * 128, :] = _ln(X[c * 128:(c + 1) * 128, :].astype(f32)).astype(bf16)
    for cp in w_copies(0):
        cp.wait()

    lane128 = lax.broadcasted_iota(i32, (QB // 2, 128), 1) >> 5

    def proj_chunk(c, par, g, slot):
        rows = slice(c * 128, (c + 1) * 128)
        kqv = _dot(XN[par, rows, :], W3[g])
        k = kqv[:, 0:128]
        q = kqv[:, 128:256]
        v = kqv[:, 256:384]
        KB[slot, rows, :] = k.astype(bf16)
        PK[par * G + g, rows, :] = _phi(k).astype(bf16)
        QS[slot, rows, :] = (q * QSCALE).astype(bf16)
        PQ[slot, rows, :] = _phi(q).astype(bf16)
        VT[par * G + g, 0:128, rows] = v.astype(bf16).T

    def mem_update(par, g):
        prev = (1 - par) * G + g
        MEM[g] = MEM[g] + _dot(VT[prev], PK[prev])

    def mem_read(g, slot):
        return _dot_nt((MEM[g] * MMASK[...]).astype(bf16), PQ[slot])

    def qk(i, slot):
        n = QB * (i + 1)
        qi = pltpu.bitcast(QS[slot, i * QB:(i + 1) * QB, :], jnp.uint32)
        qm = jnp.concatenate(
            [pltpu.bitcast(jnp.where(lane128 == h, qi, jnp.uint32(0)), bf16) for h in range(HG)], axis=0)
        return _dot_nt(KB[slot, 0:n, :], qm)

    def softmax(i, st):
        n = QB * (i + 1)
        ps = []
        for h in range(HG):
            sh = st[:, h * QB:(h + 1) * QB]
            sd = sh[n - QB:, :] + MASK[...]
            sh = sd if i == 0 else jnp.concatenate([sh[:n - QB, :], sd], axis=0)
            m = jnp.max(sh, axis=0, keepdims=True)
            p = jnp.exp2(sh - m)
            ps.append((p.astype(bf16), _colsum(p)))
        return ps

    def pv(i, ps, mrd, par, g):
        n = QB * (i + 1)
        outs = []
        for h in range(HG):
            p, l = ps[h]
            o = _dot(VT[par * G + g, h * DH:(h + 1) * DH, 0:n], p)
            gt = GATE[pl.ds(g * HG + h, 1), :]
            o = o * ((1.0 - gt) / l)
            if mrd is not None:
                num = mrd[h * DH:(h + 1) * DH, i * QB:(i + 1) * QB]
                den = mrd[128 + h:129 + h, i * QB:(i + 1) * QB] + 1e-6
                o = num * (gt / den) + o
            outs.append(o)
        ot = jnp.concatenate(outs, axis=0)
        OB[par * G + g, i * QB:(i + 1) * QB, :] = ot.T.astype(bf16)

    def wo_rows(par, r0, n):
        o = jnp.concatenate([OB[par * G + g, pl.ds(r0, n), :] for g in range(G)], axis=1)
        return _dot(o, WO[...])

    def post_rows(y, row0, n):
        rows = pl.ds(row0, n)
        x1 = _rbf(X[rows, :].astype(f32) + _rbf(y))
        xb16 = _ln(x1).astype(bf16)
        xb = xb16.astype(f32)
        XB[rows, :] = xb16
        X[rows, :] = (x1 + xb).astype(bf16)
        r = _rbf(jnp.sum(xb * WR[0:1, :], axis=1, keepdims=True))
        bits = pltpu.bitcast(jnp.broadcast_to(r, (n, 128)), i32)
        key = bits ^ ((bits >> 31) & 0x7FFF0000)
        key = key | (S - 1 - row0 - lax.broadcasted_iota(i32, (n, 128), 0))
        t1 = TOP[0:8, :]
        t2 = TOP[8:16, :]
        for j in range(n // 8):
            kj = key[j * 8:(j + 1) * 8]
            t2 = jnp.maximum(t2, jnp.minimum(t1, kj))
            t1 = jnp.maximum(t1, kj)
        TOP[0:8, :] = t1
        TOP[8:16, :] = t2

    def ln_a(par, s_src, r0, n):
        src = pl.ds(pl.multiple_of(s_src * L + r0, 16), n)
        XN[par, pl.ds(r0, n), :] = _ln(X[src, :].astype(f32)).astype(bf16)

    def group_iter(s, g, slot, first_seg, nxt):
        par = s % 2
        r0 = pl.multiple_of(g * CH, CH)
        npar, ng = nxt
        if not first_seg:
            mem_update(par, g)
        st3 = qk(3, slot)
        proj_chunk(0, npar, ng, 1 - slot)
        mrd = None if first_seg else mem_read(g, slot)
        p3 = softmax(3, st3)
        st2 = qk(2, slot)
        pv(3, p3, mrd, par, g)
        proj_chunk(1, npar, ng, 1 - slot)
        p2 = softmax(2, st2)
        st1 = qk(1, slot)
        pv(2, p2, mrd, par, g)
        if not first_seg:
            y = wo_rows(1 - par, r0, CH)
        p1 = softmax(1, st1)
        st0 = qk(0, slot)
        pv(1, p1, mrd, par, g)
        proj_chunk(2, npar, ng, 1 - slot)
        p0 = softmax(0, st0)
        pv(0, p0, mrd, par, g)
        if not first_seg:
            post_rows(y, pl.multiple_of((s - 1) * L + r0, CH), CH)
        ln_a(1 - par, (s + 1) % NSEG, r0, CH)
        proj_chunk(3, npar, ng, 1 - slot)

    def tail():
        s = NSEG - 1
        par = s % 2
        for g in range(G - U, G - 1):
            group_iter(s, g, g % 2, False, (par, g + 1))
        g = G - 1
        slot = g % 2
        r0 = g * CH
        mem_update(par, g)
        st3 = qk(3, slot)
        y = wo_rows(1 - par, r0, CH)
        mrd = mem_read(g, slot)
        p3 = softmax(3, st3)
        st2 = qk(2, slot)
        pv(3, p3, mrd, par, g)
        post_rows(y, (s - 1) * L + r0, CH)
        p2 = softmax(2, st2)
        st1 = qk(1, slot)
        pv(2, p2, mrd, par, g)
        y3 = wo_rows(par, 3 * QB, QB)
        p1 = softmax(1, st1)
        st0 = qk(0, slot)
        pv(1, p1, mrd, par, g)
        ln_a(1 - par, 0, r0, CH)
        y2 = wo_rows(par, 2 * QB, QB)
        p0 = softmax(0, st0)
        pv(0, p0, mrd, par, g)
        post_rows(y3, s * L + 3 * QB, QB)
        y1 = wo_rows(par, QB, QB)
        post_rows(y2, s * L + 2 * QB, QB)
        y0 = wo_rows(par, 0, QB)
        post_rows(y1, s * L + QB, QB)
        post_rows(y0, s * L, QB)

    def ffn():
        t = TOP[...]
        k1 = jnp.max(t, axis=0, keepdims=True)
        k2 = jnp.max(jnp.where(t == k1, IMIN, t), axis=0, keepdims=True)
        sub = lax.broadcasted_iota(i32, (16, D), 0)
        idx, blks, sgs = [], [], []
        for kk in (k1, k2):
            ii = jnp.clip(S - 1 - (jnp.max(kk) & 0xFFFF), 0, S - 1)
            hi = kk & (-65536)
            rv = pltpu.bitcast(hi ^ ((hi >> 31) & 0x7FFF0000), f32)
            sgs.append(_rbf(_sigmoid(rv))[:, 0:1])
            idx.append(ii)
            blks.append(XB[pl.ds(pl.multiple_of((ii >> 4) << 4, 16), 16), :])
        xs = jnp.concatenate(blks, axis=0)
        gt = _rbf(_dot(xs, WG[...]))
        up = _rbf(_dot(xs, WU[...]))
        hh = (_rbf(gt * _sigmoid(gt)) * up).astype(bf16)
        nk = 4
        kc = F // nk
        y = _dot(hh[:, 0:kc], WD[0:kc, :])
        for j in range(1, nk):
            y = y + _dot(hh[:, j * kc:(j + 1) * kc], WD[j * kc:(j + 1) * kc, :])
        y = _rbf(y)
        return idx, [_rbf(y[j * 16:(j + 1) * 16, :] * sgs[j]) for j in range(2)], sub

    def patch(idx, ys, sub):
        for ii, yj in zip(idx, ys):
            b = pl.multiple_of((ii >> 4) << 4, 16)
            blk = X[pl.ds(b, 16), :].astype(f32)
            X[pl.ds(b, 16), :] = jnp.where(sub == (ii & 15), blk + yj, blk).astype(bf16)

    def layer_body(layer, carry):
        MEM[...] = jnp.zeros(MEM.shape, f32)
        TOP[...] = jnp.full(TOP.shape, IMIN, i32)
        for c in range(4):
            proj_chunk(c, 0, 0, 0)

        def body_a(j, c):
            @pl.when(layer == 0)
            def _():
                for u in range(U):
                    g = j * U + u + 1

                    @pl.when(g < G)
                    def _():
                        for cp in w_copies(g):
                            cp.wait()

                    @pl.when(g + U < G)
                    def _():
                        for cp in w_copies(g + U):
                            cp.start()

                @pl.when(j == 0)
                def _():
                    x_copy(1).wait()

                @pl.when(j == 1)
                def _():
                    wo_copy.start()
                    x_copy(2).start()
                    x_copy(3).start()

            for u in range(U):
                g = j * U + u
                if u < U - 1:
                    nxt = (0, g + 1)
                else:
                    nxt = (jnp.where(j == G // U - 1, 1, 0), (g + 1) % G)
                group_iter(0, g, u % 2, True, nxt)
            return c

        lax.fori_loop(0, G // U, body_a, 0)

        @pl.when(layer == 0)
        def _():
            wo_copy.wait()
            x_copy(2).wait()
            x_copy(3).wait()
            wg_copy.start()
            wu_copy.start()
            wd_copy.start()

        def body_b(it, c):
            s = 1 + it // (G // U)
            j = it % (G // U)
            for u in range(U):
                g = j * U + u
                if u < U - 1:
                    nxt = (s % 2, g + 1)
                else:
                    nxt = ((s + jnp.where(j == G // U - 1, 1, 0)) % 2, (g + 1) % G)
                group_iter(s, g, u % 2, False, nxt)

            @pl.when(jnp.logical_and(layer == 1, j == G // U - 1))
            def _():
                out_copy(s - 1).start()

            return c

        lax.fori_loop(0, 3 * (G // U) - 1, body_b, 0)
        tail()

        @pl.when(layer == 0)
        def _():
            wg_copy.wait()
            wu_copy.wait()
            wd_copy.wait()

        @pl.when(layer == 1)
        def _():
            out_copy(NSEG - 2).start()
            out_copy(NSEG - 1).start()

        idx, ys, sub = ffn()

        @pl.when(layer == 1)
        def _():
            for s in range(NSEG):
                out_copy(s).wait()

        patch(idx, ys, sub)

        @pl.when(layer == 0)
        def _():
            for ii in idx:
                @pl.when(ii < L)
                def _():
                    ln_a(0, 0, pl.multiple_of((ii >> 4) << 4, 16), 16)

        @pl.when(layer == 1)
        def _():
            bs = [pl.multiple_of((ii >> 4) << 4, 16) for ii in idx]
            cps = [pltpu.make_async_copy(X.at[pl.ds(b, 16), :], out_hbm.at[0, pl.ds(b, 16), :], sem_o.at[j])
                   for j, b in enumerate(bs)]
            cps[0].start()

            @pl.when(bs[0] != bs[1])
            def _():
                cps[1].start()
                cps[1].wait()

            cps[0].wait()

        return carry

    lax.fori_loop(0, 2, layer_body, 0)


@jax.jit
def pallas_interleave_layers__memory_aug_infini_attn__moe_arch_mod__prompt_kernel(
    A_x: jax.Array,
    A_wq: jax.Array,
    A_wk: jax.Array,
    A_wv: jax.Array,
    A_wo: jax.Array,
    A_beta: jax.Array,
    B_x: jax.Array,
    B_w_r: jax.Array,
    B_w_gate: jax.Array,
    B_w_up: jax.Array,
    B_w_down: jax.Array,
):
    del B_x
    any_spec = pl.BlockSpec(memory_space=pl.ANY)
    vmem_spec = pl.BlockSpec(memory_space=pltpu.VMEM)
    scratch = [
        pltpu.VMEM((S, D), bf16),
        pltpu.VMEM((S, D), bf16),
        pltpu.VMEM((2, L, D), bf16),
        pltpu.VMEM((G, D, 384), bf16),
        pltpu.VMEM((D, D), bf16),
        pltpu.VMEM((D, F), bf16),
        pltpu.VMEM((D, F), bf16),
        pltpu.VMEM((F, D), bf16),
        pltpu.VMEM((2, L, 128), bf16),
        pltpu.VMEM((2, L, 128), bf16),
        pltpu.VMEM((2, L, 128), bf16),
        pltpu.VMEM((2 * G, L, 128), bf16),
        pltpu.VMEM((2 * G, MR, L), bf16),
        pltpu.VMEM((2 * G, L, 128), bf16),
        pltpu.VMEM((G, MR, 128), f32),
        pltpu.VMEM((16, 128), i32),
        pltpu.VMEM((H, 128), f32),
        pltpu.VMEM((128, 128), f32),
        pltpu.VMEM((MR, 128), f32),
        pltpu.VMEM((8, D), f32),
        pltpu.SemaphoreType.DMA((NSEG + 4,)),
        pltpu.SemaphoreType.DMA((3 * G + 1,)),
        pltpu.SemaphoreType.DMA((3,)),
        pltpu.SemaphoreType.DMA((NSEG,)),
    ]
    return pl.pallas_call(
        _kernel,
        out_shape=jax.ShapeDtypeStruct((1, S, D), bf16),
        in_specs=[any_spec, any_spec, any_spec, any_spec, any_spec, vmem_spec, vmem_spec,
                  any_spec, any_spec, any_spec],
        out_specs=any_spec,
        scratch_shapes=scratch,
        compiler_params=pltpu.CompilerParams(vmem_limit_bytes=100 * 2 ** 20),
    )(A_x, A_wq, A_wk, A_wv, A_wo, A_beta.reshape(1, H), B_w_r.reshape(1, D), B_w_gate, B_w_up, B_w_down)
```

```python
import functools
import math

import jax
import jax.numpy as jnp
from jax import lax
import jax.experimental.pallas as pl
import jax.experimental.pallas.tpu as pltpu

S = 2048
D = 1024
H = 32
DH = 32
NSEG = 4
L = S // NSEG
F = 3584
G = 8
HG = 4
QB = 128
NQB = L // QB
MR = 144
CH = L // G
U = 2
PD = 16
PE = 4
EPS = 1e-5
LOG2E = math.log2(math.e)
QSCALE = (DH ** -0.5) * LOG2E
NEG = -1e9 * LOG2E
IMIN = -2 ** 31

f32 = jnp.float32
bf16 = jnp.bfloat16
i32 = jnp.int32
u32 = jnp.uint32

NT = (((1,), (1,)), ((), ()))


def _rbf(x):
    return x.astype(bf16).astype(f32)


def _ln(x):
    m = jnp.sum(x, axis=1, keepdims=True) * (1.0 / D)
    mb = _rbf(m)
    c = x - mb
    e = m - mb
    v = jnp.maximum(jnp.sum(c * c, axis=1, keepdims=True) * (1.0 / D) - e * e, 0.0)
    sd = _rbf(jnp.sqrt(_rbf(_rbf(v) + EPS)))
    return c * (1.0 / sd)


def _phi(t):
    return jnp.where(t > 0, t + 1.0, jnp.exp(t))


def _sigmoid(t):
    return 1.0 / (1.0 + jnp.exp(-t))


def _dot(a, b):
    return jnp.dot(a, b, preferred_element_type=f32)


def _dot_nt(a, b):
    return lax.dot_general(a, b, NT, preferred_element_type=f32)


def _ds(start, size, mult):
    if isinstance(start, int):
        return pl.ds(start, size)
    return pl.ds(pl.multiple_of(start, mult), size)


def _colred(p, op, nacc=2):
    n = p.shape[0]
    parts = [p[j * 8:(j + 1) * 8] for j in range(n // 8)]
    acc = parts[:nacc]
    for j in range(nacc, len(parts)):
        acc[j % nacc] = op(acc[j % nacc], parts[j])
    r = acc[0]
    for a in acc[1:]:
        r = op(r, a)
    return r


def _kernel(x_hbm, wq_hbm, wk_hbm, wv_hbm, wo_hbm, beta_ref, wr_ref, wg_hbm, wu_hbm, wd_hbm,
            out_hbm,
            X, XB, XN, W3, WO, WG, WU, WD,
            KB, QS, PQ, VT, PKS, VTS, OB, MEMB, PB0, PB1, PB2, PB3,
            SC0, SC1, SC2, SC3, MEM, TOP, GATE, MASK, MMASK, WR, ZS,
            sem_x, sem_w, sem_f, sem_o):
    X, XB, XN, W3, WO, WG, WU, WD, KB, QS, PQ, VT, PKS, VTS, OB, MEMB, PB0, PB1, PB2, PB3 = [
        r.bitcast(bf16) for r in
        (X, XB, XN, W3, WO, WG, WU, WD, KB, QS, PQ, VT, PKS, VTS, OB, MEMB, PB0, PB1, PB2, PB3)]
    PB = (PB0, PB1, PB2, PB3)
    SC = (SC0, SC1, SC2, SC3)

    def x0_copy(c):
        return pltpu.make_async_copy(x_hbm.at[0, pl.ds(c * 128, 128), :], X.at[pl.ds(c * 128, 128), :],
                                     sem_x.at[NSEG + c])

    def x_copy(s):
        return pltpu.make_async_copy(x_hbm.at[0, pl.ds(s * L, L), :], X.at[pl.ds(s * L, L), :], sem_x.at[s])

    def w_copies(g):
        col = pl.multiple_of(g * 128, 128)
        return [pltpu.make_async_copy(w.at[:, pl.ds(col, 128)], W3.at[g, :, pl.ds(j * 128, 128)],
                                      sem_w.at[3 * g + j])
                for j, w in enumerate((wk_hbm, wq_hbm, wv_hbm))]

    wo_copy = pltpu.make_async_copy(wo_hbm, WO, sem_w.at[3 * G])
    wg_copy = pltpu.make_async_copy(wg_hbm, WG, sem_f.at[0])
    wu_copy = pltpu.make_async_copy(wu_hbm, WU, sem_f.at[1])
    wd_copy = pltpu.make_async_copy(wd_hbm, WD, sem_f.at[2])

    def out_copy(s):
        base = pl.multiple_of(s * L, L)
        return pltpu.make_async_copy(X.at[pl.ds(base, L), :], out_hbm.at[0, pl.ds(base, L), :], sem_o.at[s])

    x0_copy(0).start()
    for cp in w_copies(0):
        cp.start()
    for c in range(1, 4):
        x0_copy(c).start()
    for g in range(1, 1 + U):
        for cp in w_copies(g):
            cp.start()
    x_copy(1).start()

    row = lax.broadcasted_iota(i32, (128, 128), 0)
    col = lax.broadcasted_iota(i32, (128, 128), 1)
    MASK[...] = jnp.where(row > col, NEG, 0.0).astype(f32)
    r144 = lax.broadcasted_iota(i32, (MR, 128), 0)
    c144 = lax.broadcasted_iota(i32, (MR, 128), 1)
    head_of_row = jnp.where(r144 < 128, r144 >> 5, r144 - 128)
    MMASK[...] = jnp.where(head_of_row == (c144 >> 5), 1.0, 0.0).astype(f32)
    for t in range(2 * G):
        VTS[t * MR + 128:(t + 1) * MR, :] = jnp.ones((MR - 128, L), bf16)
    ZS[0] = 0
    gsig = _rbf(_sigmoid(beta_ref[...].astype(f32)))
    r32 = lax.broadcasted_iota(i32, (H, H), 0)
    c32 = lax.broadcasted_iota(i32, (H, H), 1)
    gcol = jnp.sum(jnp.where(r32 == c32, jnp.broadcast_to(gsig, (H, H)), 0.0), axis=1, keepdims=True)
    GATE[...] = jnp.broadcast_to(gcol, (H, 128))
    WR[...] = jnp.broadcast_to(wr_ref[...].astype(f32), (8, D))

    for c in range(L // 128):
        x0_copy(c).wait()
        XN[c * 128:(c + 1) * 128, :] = _ln(X[c * 128:(c + 1) * 128, :].astype(f32)).astype(bf16)
    for cp in w_copies(0):
        cp.wait()

    lane128 = lax.broadcasted_iota(i32, (QB // 2, 128), 1) >> 5

    def proj_chunk(c, par, g, slot):
        rows = slice(c * 128, (c + 1) * 128)
        srows = slice(slot * L + c * 128, slot * L + (c + 1) * 128)
        item = par * G + g
        kqv = _dot(XN[_ds(par * L + c * 128, 128, 128), :], W3[g])
        k = kqv[:, 0:128]
        q = kqv[:, 128:256]
        v = kqv[:, 256:384]
        KB[srows, 0:128] = k.astype(bf16)
        PKS[_ds(item * L + c * 128, 128, 128), 0:128] = _phi(k).astype(bf16)
        QS[srows, 0:128] = (q * QSCALE).astype(bf16)
        PQ[srows, 0:128] = _phi(q).astype(bf16)
        vt = v.astype(bf16).T
        VT[slot * 128:(slot + 1) * 128, rows] = vt
        VTS[_ds(item * MR, 128, 16), rows] = vt

    def mem_update(par, g):
        prev = (1 - par) * G + g
        m = MEM[g] + _dot(VTS[_ds(prev * MR, MR, 16), :], PKS[_ds(prev * L, L, L), 0:128])
        MEM[g] = m
        MEMB[:, 0:128] = (m * MMASK[...]).astype(bf16)

    def qk(i, slot):
        n = QB * (i + 1)
        qi = pltpu.bitcast(QS[slot * L + i * QB:slot * L + (i + 1) * QB, 0:128], u32)
        qm = jnp.concatenate(
            [pltpu.bitcast(jnp.where(lane128 == h, qi, jnp.uint32(0)), bf16) for h in range(HG)], axis=0)
        st = _dot_nt(KB[slot * L:slot * L + n, 0:128], qm)
        ms = []
        for h in range(HG):
            sh = st[:, h * QB:(h + 1) * QB]
            sd = sh[n - QB:, :] + MASK[...]
            sh = sd if i == 0 else jnp.concatenate([sh[:n - QB, :], sd], axis=0)
            SC[i][:, h * QB:(h + 1) * QB] = sh
            ms.append(jnp.max(_colred(sh, jnp.maximum), axis=0, keepdims=True))
        return ms

    def expo(i, ms):
        ls = []
        n = QB * (i + 1)
        z = ZS[0]
        hist = []
        for h in range(HG):
            a = SC[i][_ds(z, n, 8), h * QB:(h + 1) * QB] - ms[h]
            ps = []
            acc = [None, None]
            for k in range(n // 8):
                ak = a[k * 8:(k + 1) * 8]
                if len(hist) >= PD and k % PE < 2:
                    ak = jnp.minimum(ak, hist[-PD])
                pk = jnp.exp2(ak)
                acc[k % 2] = pk if acc[k % 2] is None else acc[k % 2] + pk
                hist.append(acc[k % 2])
                ps.append(pk)
            PB[i][:, h * QB:(h + 1) * QB] = jnp.concatenate(ps, axis=0).astype(bf16)
            ls.append(jnp.sum(acc[0] + acc[1], axis=0, keepdims=True))
        return ls

    def pv(i, ls, use_mem, par, g, slot):
        n = QB * (i + 1)
        if use_mem:
            mrd = _dot_nt(MEMB[:, 0:128], PQ[slot * L + i * QB:slot * L + (i + 1) * QB, 0:128])
        outs = []
        z = ZS[0]
        for h in range(HG):
            o = _dot(VT[slot * 128 + h * DH:slot * 128 + (h + 1) * DH, 0:n], PB[i][_ds(z, n, 16), h * QB:(h + 1) * QB])
            gt = GATE[pl.ds(g * HG + h, 1), :]
            o = o * ((1.0 - gt) / ls[h])
            if use_mem:
                num = mrd[h * DH:(h + 1) * DH, :]
                den = mrd[128 + h:129 + h, :] + 1e-6
                o = num * (gt / den) + o
            outs.append(o)
        ot = jnp.concatenate(outs, axis=0)
        OB[_ds((par * G + g) * L + i * QB, QB, QB), 0:128] = ot.astype(bf16).T

    def wo_rows(par, r0, row0, n):
        o = jnp.concatenate([OB[_ds((par * G + g) * L + r0, n, 16), 0:128] for g in range(G)], axis=1)
        y = _dot(o, WO[...])
        rows = pl.ds(row0, n)
        X[rows, :] = (X[rows, :].astype(f32) + _rbf(y)).astype(bf16)

    def post_rows(row0, n):
        rows = pl.ds(row0, n)
        x1 = X[rows, :].astype(f32)
        xb16 = _ln(x1).astype(bf16)
        xb = xb16.astype(f32)
        XB[rows, :] = xb16
        X[rows, :] = (x1 + xb).astype(bf16)
        r = _rbf(jnp.sum(xb * WR[0:1, :], axis=1, keepdims=True))
        bits = pltpu.bitcast(jnp.broadcast_to(r, (n, 128)), i32)
        key = bits ^ ((bits >> 31) & 0x7FFF0000)
        key = key | (S - 1 - row0 - lax.broadcasted_iota(i32, (n, 128), 0))
        t1 = TOP[0:8, :]
        t2 = TOP[8:16, :]
        for j in range(n // 8):
            kj = key[j * 8:(j + 1) * 8]
            t2 = jnp.maximum(t2, jnp.minimum(t1, kj))
            t1 = jnp.maximum(t1, kj)
        TOP[0:8, :] = t1
        TOP[8:16, :] = t2

    def ln_a(par, s_src, r0, n):
        src = pl.ds(pl.multiple_of(s_src * L + r0, 16), n)
        XN[_ds(par * L + r0, n, 16), :] = _ln(X[src, :].astype(f32)).astype(bf16)

    def group_iter(s, g, slot, first_seg, nxt, ln):
        par = s % 2
        r0 = pl.multiple_of(g * CH, CH)
        mem = not first_seg
        last = nxt is None
        if last:
            P = lambda c: None
        else:
            P = lambda c: proj_chunk(c, nxt[0], nxt[1], 1 - slot)
        if mem:
            row0 = pl.multiple_of((s - 1) * L + r0, CH)
            wo_rows(1 - par, r0, row0, CH)
            mem_update(par, g)
        m3 = qk(3, slot)
        if mem:
            post_rows(row0, CH)
        P(0)
        l3 = expo(3, m3)
        m2 = qk(2, slot)
        pv(3, l3, mem, par, g, slot)
        if last:
            wo_rows(par, 3 * QB, s * L + 3 * QB, QB)
        P(1)
        l2 = expo(2, m2)
        m1 = qk(1, slot)
        pv(2, l2, mem, par, g, slot)
        m0 = qk(0, slot)
        if last:
            wo_rows(par, 2 * QB, s * L + 2 * QB, QB)
            post_rows(s * L + 3 * QB, QB)
        P(2)
        l1 = expo(1, m1)
        l0 = expo(0, m0)
        pv(1, l1, mem, par, g, slot)
        pv(0, l0, mem, par, g, slot)
        P(3)
        ln_a(*ln)
        if last:
            wo_rows(par, QB, s * L + QB, QB)
            post_rows(s * L + 2 * QB, QB)
            wo_rows(par, 0, s * L, QB)
            post_rows(s * L + QB, QB)
            post_rows(s * L, QB)

    def ln_item(s, g):
        wrap = (g + 1) // G
        t = s + 1 + wrap
        return (t % 2, t % NSEG, pl.multiple_of(((g + 1) % G) * CH, CH), CH)

    def ffn():
        t = TOP[...]
        k1 = jnp.max(t, axis=0, keepdims=True)
        k2 = jnp.max(jnp.where(t == k1, IMIN, t), axis=0, keepdims=True)
        sub = lax.broadcasted_iota(i32, (16, D), 0)
        idx, blks, sgs = [], [], []
        for kk in (k1, k2):
            ii = jnp.clip(S - 1 - (jnp.max(kk) & 0xFFFF), 0, S - 1)
            hi = kk & (-65536)
            rv = pltpu.bitcast(hi ^ ((hi >> 31) & 0x7FFF0000), f32)
            sgs.append(_rbf(_sigmoid(rv))[:, 0:1])
            idx.append(ii)
            blks.append(XB[pl.ds(pl.multiple_of((ii >> 4) << 4, 16), 16), :])
        xs = jnp.concatenate(blks, axis=0)
        gt = _rbf(_dot(xs, WG[...]))
        up = _rbf(_dot(xs, WU[...]))
        hh = (_rbf(gt * _sigmoid(gt)) * up).astype(bf16)
        nk = 4
        kc = F // nk
        y = _dot(hh[:, 0:kc], WD[0:kc, :])
        for j in range(1, nk):
            y = y + _dot(hh[:, j * kc:(j + 1) * kc], WD[j * kc:(j + 1) * kc, :])
        y = _rbf(y)
        return idx, [_rbf(y[j * 16:(j + 1) * 16, :] * sgs[j]) for j in range(2)], sub

    def patch(idx, ys, sub):
        for ii, yj in zip(idx, ys):
            b = pl.multiple_of((ii >> 4) << 4, 16)
            blk = X[pl.ds(b, 16), :].astype(f32)
            X[pl.ds(b, 16), :] = jnp.where(sub == (ii & 15), blk + yj, blk).astype(bf16)

    def layer_body(layer, carry):
        MEM[...] = jnp.zeros(MEM.shape, f32)
        TOP[...] = jnp.full(TOP.shape, IMIN, i32)
        for c in range(4):
            proj_chunk(c, 0, 0, 0)

        @pl.when(layer == 0)
        def _():
            x_copy(1).wait()

        ln_a(1, 1, 0, CH)

        def body_a(j, c):
            @pl.when(layer == 0)
            def _():
                for u in range(U):
                    g = j * U + u + 1

                    @pl.when(g < G)
                    def _():
                        for cp in w_copies(g):
                            cp.wait()

                    @pl.when(g + U < G)
                    def _():
                        for cp in w_copies(g + U):
                            cp.start()

                @pl.when(j == 1)
                def _():
                    wo_copy.start()
                    x_copy(2).start()
                    x_copy(3).start()

                @pl.when(j == G // U - 1)
                def _():
                    x_copy(2).wait()

            for u in range(U):
                g = j * U + u
                if u < U - 1:
                    nxt = (0, g + 1)
                else:
                    nxt = (jnp.where(j == G // U - 1, 1, 0), (g + 1) % G)
                group_iter(0, g, u % 2, True, nxt, ln_item(0, g))
            return c

        lax.fori_loop(0, G // U, body_a, 0)

        @pl.when(layer == 0)
        def _():
            wo_copy.wait()
            x_copy(3).wait()
            wg_copy.start()
            wu_copy.start()
            wd_copy.start()

        def body_b(it, c):
            s = 1 + it // (G // U)
            j = it % (G // U)
            for u in range(U):
                g = j * U + u
                if u < U - 1:
                    nxt = (s % 2, g + 1)
                else:
                    nxt = ((s + jnp.where(j == G // U - 1, 1, 0)) % 2, (g + 1) % G)
                group_iter(s, g, u % 2, False, nxt, ln_item(s, g))

            @pl.when(jnp.logical_and(layer == 1, j == G // U - 1))
            def _():
                out_copy(s - 1).start()

            return c

        lax.fori_loop(0, 3 * (G // U) - 1, body_b, 0)
        s = NSEG - 1
        for g in range(G - U, G):
            group_iter(s, g, g % 2, False, (s % 2, g + 1) if g < G - 1 else None,
                       ln_item(s, g) if g < G - 1 else (0, 0, 0, CH))

        @pl.when(layer == 0)
        def _():
            wg_copy.wait()
            wu_copy.wait()
            wd_copy.wait()

        @pl.when(layer == 1)
        def _():
            out_copy(NSEG - 2).start()
            out_copy(NSEG - 1).start()

        idx, ys, sub = ffn()

        @pl.when(layer == 1)
        def _():
            for s in range(NSEG):
                out_copy(s).wait()

        patch(idx, ys, sub)

        @pl.when(layer == 0)
        def _():
            for ii in idx:
                @pl.when(ii < L)
                def _():
                    ln_a(0, 0, pl.multiple_of((ii >> 4) << 4, 16), 16)

        @pl.when(layer == 1)
        def _():
            bs = [pl.multiple_of((ii >> 4) << 4, 16) for ii in idx]
            cps = [pltpu.make_async_copy(X.at[pl.ds(b, 16), :], out_hbm.at[0, pl.ds(b, 16), :], sem_o.at[j])
                   for j, b in enumerate(bs)]
            cps[0].start()

            @pl.when(bs[0] != bs[1])
            def _():
                cps[1].start()
                cps[1].wait()

            cps[0].wait()

        return carry

    lax.fori_loop(0, 2, layer_body, 0)


def _pk(*shape):
    return pltpu.VMEM((*shape[:-2], shape[-2] // 2, shape[-1]), u32)


@jax.jit
def pallas_interleave_layers__memory_aug_infini_attn__moe_arch_mod__prompt_kernel(
    A_x: jax.Array,
    A_wq: jax.Array,
    A_wk: jax.Array,
    A_wv: jax.Array,
    A_wo: jax.Array,
    A_beta: jax.Array,
    B_x: jax.Array,
    B_w_r: jax.Array,
    B_w_gate: jax.Array,
    B_w_up: jax.Array,
    B_w_down: jax.Array,
):
    del B_x
    any_spec = pl.BlockSpec(memory_space=pl.ANY)
    vmem_spec = pl.BlockSpec(memory_space=pltpu.VMEM)
    scratch = [
        _pk(S, D),
        _pk(S, D),
        _pk(2 * L, D),
        _pk(G, D, 384),
        _pk(D, D),
        _pk(D, F),
        _pk(D, F),
        _pk(F, D),
        _pk(2 * L, 256),
        _pk(2 * L, 256),
        _pk(2 * L, 256),
        _pk(2 * 128, L),
        _pk(2 * G * L, 256),
        _pk(2 * G * MR, L),
        _pk(2 * G * L, 256),
        _pk(MR, 256),
        _pk(QB, 512), _pk(2 * QB, 512), _pk(3 * QB, 512), _pk(4 * QB, 512),
        pltpu.VMEM((QB, 512), f32), pltpu.VMEM((2 * QB, 512), f32),
        pltpu.VMEM((3 * QB, 512), f32), pltpu.VMEM((4 * QB, 512), f32),
        pltpu.VMEM((G, MR, 128), f32),
        pltpu.VMEM((16, 128), i32),
        pltpu.VMEM((H, 128), f32),
        pltpu.VMEM((128, 128), f32),
        pltpu.VMEM((MR, 128), f32),
        pltpu.VMEM((8, D), f32),
        pltpu.SMEM((1,), i32),
        pltpu.SemaphoreType.DMA((NSEG + 4,)),
        pltpu.SemaphoreType.DMA((3 * G + 1,)),
        pltpu.SemaphoreType.DMA((3,)),
        pltpu.SemaphoreType.DMA((NSEG,)),
    ]
    return pl.pallas_call(
        _kernel,
        out_shape=jax.ShapeDtypeStruct((1, S, D), bf16),
        in_specs=[any_spec, any_spec, any_spec, any_spec, any_spec, vmem_spec, vmem_spec,
                  any_spec, any_spec, any_spec],
        out_specs=any_spec,
        scratch_shapes=scratch,
        compiler_params=pltpu.CompilerParams(vmem_limit_bytes=100 * 2 ** 20),
    )(A_x, A_wq, A_wk, A_wv, A_wo, A_beta.reshape(1, H), B_w_r.reshape(1, D), B_w_gate, B_w_up, B_w_down)
```

```python
import functools
import math

import jax
import jax.numpy as jnp
from jax import lax
import jax.experimental.pallas as pl
import jax.experimental.pallas.tpu as pltpu

S = 2048
D = 1024
H = 32
DH = 32
NSEG = 4
L = S // NSEG
F = 3584
G = 8
HG = 4
QB = 128
NQB = L // QB
MR = 144
CH = L // G
U = 2
SB = 32
PD = 16
PE = 4
XBO = S + CH
EPS = 1e-5
LOG2E = math.log2(math.e)
QSCALE = (DH ** -0.5) * LOG2E
NEG = -1e9 * LOG2E
IMIN = -2 ** 31

f32 = jnp.float32
bf16 = jnp.bfloat16
i32 = jnp.int32
u32 = jnp.uint32

NT = (((1,), (1,)), ((), ()))


def _rbf(x):
    return x.astype(bf16).astype(f32)


def _ln(x):
    m = jnp.sum(x, axis=1, keepdims=True) * (1.0 / D)
    mb = _rbf(m)
    c = x - mb
    e = m - mb
    v = jnp.maximum(jnp.sum(c * c, axis=1, keepdims=True) * (1.0 / D) - e * e, 0.0)
    sd = _rbf(jnp.sqrt(_rbf(_rbf(v) + EPS)))
    return c * (1.0 / sd)


def _phi(t):
    return jnp.where(t > 0, t + 1.0, jnp.exp(t))


def _sigmoid(t):
    return 1.0 / (1.0 + jnp.exp(-t))


def _dot(a, b):
    return jnp.dot(a, b, preferred_element_type=f32)


def _dot_nt(a, b):
    return lax.dot_general(a, b, NT, preferred_element_type=f32)


def _ds(start, size, mult):
    if isinstance(start, int):
        return pl.ds(start, size)
    return pl.ds(pl.multiple_of(start, mult), size)


def _colred(p, op, nacc=2):
    n = p.shape[0]
    parts = [p[j * 8:(j + 1) * 8] for j in range(n // 8)]
    acc = parts[:nacc]
    for j in range(nacc, len(parts)):
        acc[j % nacc] = op(acc[j % nacc], parts[j])
    r = acc[0]
    for a in acc[1:]:
        r = op(r, a)
    return r


def _kernel(x_hbm, wq_hbm, wk_hbm, wv_hbm, wo_hbm, beta_ref, wr_ref, wg_hbm, wu_hbm, wd_hbm,
            out_hbm,
            X, XN, LS, W3, WO, WG, WU, WD,
            KB, QS, PQ, VT, PKS, VTS, OB, MEMB, PB0, PB1, PB2, PB3, YB, OS0, OS1, OS2, OS3,
            SC0, SC1, SC2, SC3, MEM, TOP, GATE, MASK, MMASK, WR, ZS,
            sem_x, sem_w, sem_f, sem_o):
    X, XN, LS, W3, WO, WG, WU, WD, KB, QS, PQ, VT, PKS, VTS, OB, MEMB, YB = [
        r.bitcast(bf16) for r in
        (X, XN, LS, W3, WO, WG, WU, WD, KB, QS, PQ, VT, PKS, VTS, OB, MEMB, YB)]
    PB = [r.bitcast(bf16) for r in (PB0, PB1, PB2, PB3)]
    OS = [r.bitcast(bf16) for r in (OS0, OS1, OS2, OS3)]
    SC = (SC0, SC1, SC2, SC3)

    def x0_copy(c):
        return pltpu.make_async_copy(x_hbm.at[0, pl.ds(c * 128, 128), :], X.at[pl.ds(c * 128, 128), :],
                                     sem_x.at[NSEG + c])

    def x_copy(s):
        r0 = s * L + (128 if s == 1 else 0)
        n = (s + 1) * L - r0
        return pltpu.make_async_copy(x_hbm.at[0, pl.ds(r0, n), :], X.at[pl.ds(r0, n), :], sem_x.at[s])

    def w_copies(g):
        col = pl.multiple_of(g * 128, 128)
        return [pltpu.make_async_copy(w.at[:, pl.ds(col, 128)], W3.at[g, :, pl.ds(j * 128, 128)],
                                      sem_w.at[3 * g + j])
                for j, w in enumerate((wk_hbm, wq_hbm, wv_hbm))]

    wo_copy = pltpu.make_async_copy(wo_hbm, WO, sem_w.at[3 * G])
    wg_copy = pltpu.make_async_copy(wg_hbm, WG, sem_f.at[0])
    wu_copy = pltpu.make_async_copy(wu_hbm, WU, sem_f.at[1])
    wd_copy = pltpu.make_async_copy(wd_hbm, WD, sem_f.at[2])

    def out_copy(s):
        base = pl.multiple_of(s * L, L)
        return pltpu.make_async_copy(X.at[pl.ds(base, L), :], out_hbm.at[0, pl.ds(base, L), :], sem_o.at[s])

    x0_copy(0).start()
    for cp in w_copies(0):
        cp.start()
    for c in range(1, 5):
        x0_copy(c).start()
    for g in range(1, 1 + U):
        for cp in w_copies(g):
            cp.start()
    x_copy(1).start()

    row = lax.broadcasted_iota(i32, (128, 128), 0)
    col = lax.broadcasted_iota(i32, (128, 128), 1)
    MASK[...] = jnp.where(row > col, NEG, 0.0).astype(f32)
    r144 = lax.broadcasted_iota(i32, (MR, 128), 0)
    c144 = lax.broadcasted_iota(i32, (MR, 128), 1)
    head_of_row = jnp.where(r144 < 128, r144 >> 5, r144 - 128)
    MMASK[...] = jnp.where(head_of_row == (c144 >> 5), 1.0, 0.0).astype(f32)
    for t in range(2 * G):
        VTS[t * MR + 128:(t + 1) * MR, :] = jnp.ones((MR - 128, L), bf16)
    for j in range(8):
        ZS[j] = 0
    X[S:S + CH, :] = jnp.zeros((CH, D), bf16)
    for r in OS:
        r[:, 0:128] = jnp.zeros((2 * QB, 128), bf16)
    OB[2 * G * L:2 * G * L + 16, 0:128] = jnp.zeros((16, 128), bf16)
    YB[CH:2 * CH, :] = jnp.zeros((CH, D), bf16)
    gsig = _rbf(_sigmoid(beta_ref[...].astype(f32)))
    r32 = lax.broadcasted_iota(i32, (H, H), 0)
    c32 = lax.broadcasted_iota(i32, (H, H), 1)
    gcol = jnp.sum(jnp.where(r32 == c32, jnp.broadcast_to(gsig, (H, H)), 0.0), axis=1, keepdims=True)
    GATE[...] = jnp.broadcast_to(gcol, (H, 128))
    WR[...] = jnp.broadcast_to(wr_ref[...].astype(f32), (8, D))

    for c in range(L // 128):
        x0_copy(c).wait()
        XN[c * 128:(c + 1) * 128, :] = _ln(X[c * 128:(c + 1) * 128, :].astype(f32)).astype(bf16)
    for cp in w_copies(0):
        cp.wait()
    x0_copy(4).wait()

    lane128 = lax.broadcasted_iota(i32, (QB // 2, 128), 1) >> 5

    def gated(x, gate):
        if gate is None:
            return x
        xu = pltpu.bitcast(x, u32)
        top = jnp.concatenate([xu[0:8, 0:512] | jnp.concatenate([gate] * 4, axis=1), xu[0:8, 512:]], axis=1)
        return pltpu.bitcast(jnp.concatenate([top, xu[8:]], axis=0), bf16)

    def done(*vals):
        acc = None
        for v in vals:
            w = pltpu.bitcast(v, u32)
            for r in range(0, w.shape[0], 8):
                for c in range(0, w.shape[1], 128):
                    t = w[r:r + 8, c:c + 128]
                    acc = t if acc is None else acc | t
        return acc & jnp.full((8, 128), ZS[3], i32).astype(u32)

    def after(x, gate):
        if gate is None:
            return x
        xu = pltpu.bitcast(x, u32)
        return pltpu.bitcast(xu | jnp.tile(gate, (xu.shape[0] // 8, xu.shape[1] // 128)), bf16)

    def proj_part(kind, c, par, g, slot, gate=None):
        rows = slice(c * 128, (c + 1) * 128)
        srows = slice(slot * L + c * 128, slot * L + (c + 1) * 128)
        item = par * G + g
        j = 'kqv'.index(kind)
        x = XN[_ds(par * L + c * 128 + ZS[j], 128, 128), :]
        x = gated(x, gate)
        r = _dot(x, W3[g, :, j * 128:(j + 1) * 128])
        if kind == 'v':
            vt = r.astype(bf16).T
            VT[slot * 128:(slot + 1) * 128, rows] = vt
            VTS[_ds(item * MR, 128, 16), rows] = vt
            return [jnp.abs(r[t * 8:(t + 1) * 8]) for t in range(16)] + [done(vt)]
        ph = _phi(r)
        if kind == 'k':
            KB[srows, 0:128] = r.astype(bf16)
            PKS[_ds(item * L + c * 128, 128, 128), 0:128] = ph.astype(bf16)
        else:
            QS[srows, 0:128] = (r * QSCALE).astype(bf16)
            PQ[srows, 0:128] = ph.astype(bf16)
        return [ph[t * 8:(t + 1) * 8] for t in range(16)]

    def mem_update(par, g):
        prev = (1 - par) * G + g
        m = MEM[g] + _dot(VTS[_ds(prev * MR, MR, 16), :], PKS[_ds(prev * L, L, L), 0:128])
        MEM[g] = m
        MEMB[:, 0:128] = (m * MMASK[...]).astype(bf16)

    def qk(i, slot, gate=None):
        n = QB * (i + 1)
        qi = pltpu.bitcast(QS[slot * L + i * QB:slot * L + (i + 1) * QB, 0:128], u32)
        qm = jnp.concatenate(
            [pltpu.bitcast(jnp.where(lane128 == h, qi, jnp.uint32(0)), bf16) for h in range(HG)], axis=0)
        kb = KB[slot * L:slot * L + n, 0:128]
        if gate is not None:
            kb = jnp.concatenate([after(kb[0:16], gate), kb[16:]], axis=0)
        st = _dot_nt(kb, qm)
        ms = []
        for h in range(HG):
            sh = st[:, h * QB:(h + 1) * QB]
            sd = sh[n - QB:, :] + MASK[...]
            sh = sd if i == 0 else jnp.concatenate([sh[:n - QB, :], sd], axis=0)
            SC[i][:, h * QB:(h + 1) * QB] = sh
            ms.append(jnp.max(_colred(sh, jnp.maximum), axis=0, keepdims=True))
        return ms + [st[t:t + 8, 0:QB] for t in range(0, n, 64)]

    def expo(i, h, ms, hist, rel):
        n = QB * (i + 1)
        z = ZS[0]
        sc = SC[i][_ds(z, n, 8), h * QB:(h + 1) * QB]
        m = jnp.broadcast_to(ms[h], (8, QB))
        ps = []
        acc = [None, None]
        for k in range(n // 8):
            if k % PE == 0:
                pace = rel[k // PE] if rel is not None else (hist[-PD] if len(hist) >= PD else None)
                mk = m if pace is None else m + jnp.minimum(pace, 0.0)
            pk = jnp.exp2(sc[k * 8:(k + 1) * 8] - mk)
            acc[k % 2] = pk if acc[k % 2] is None else acc[k % 2] + pk
            hist.append(acc[k % 2])
            ps.append(pk)
        PB[i][:, h * QB:(h + 1) * QB] = jnp.concatenate(ps, axis=0).astype(bf16)
        return acc[0] + acc[1]

    def pv(i, ls, use_mem, par, g, slot):
        n = QB * (i + 1)
        if use_mem:
            mrd = _dot_nt(MEMB[:, 0:128], PQ[slot * L + i * QB:slot * L + (i + 1) * QB, 0:128])
        outs = []
        z = ZS[0]
        for h in range(HG):
            o = _dot(VT[slot * 128 + h * DH:slot * 128 + (h + 1) * DH, 0:n], PB[i][_ds(z, n, 16), h * QB:(h + 1) * QB])
            gt = GATE[pl.ds(g * HG + h, 1), :]
            o = o * ((1.0 - gt) / jnp.sum(ls[h], axis=0, keepdims=True))
            if use_mem:
                num = mrd[h * DH:(h + 1) * DH, :]
                den = mrd[128 + h:129 + h, :] + 1e-6
                o = num * (gt / den) + o
            outs.append(o)
        ot = jnp.concatenate(outs, axis=0)
        ot = ot.astype(bf16).T
        OS[i][slot * QB:(slot + 1) * QB, 0:128] = ot
        return done(ot)

    def flush(par, g):
        XN[_ds((1 - par) * L + g * CH, 2 * CH, 2 * CH), :] = LS[...]
        g1 = done(XN[_ds(ZS[4], 16, 16), 0:128])
        prev = (par * G + g + 2 * G - 2) % (2 * G)
        for u in range(2):
            for i in range(NQB):
                OB[_ds((prev + u) * L + i * QB, QB, QB), 0:128] = OS[i][u * QB:(u + 1) * QB, 0:128]
        return g1, done(OB[_ds(2 * G * L + ZS[4], 16, 16), 0:128])

    def wo_part(j, par, r0, y0, n, gate=None, live=None):
        o = [OB[_ds((par * G + g) * L + r0 + ZS[j], n, 16), 0:128] for g in range(G if live is None else G - 2)]
        if live is not None:
            o += [OS[r0 // QB][_ds(u * QB + r0 % QB + ZS[j], n, 16), 0:128] for u in range(2)]
        o = jnp.concatenate(o, axis=1)
        y = _dot(gated(o, gate), WO[:, j * 128:(j + 1) * 128])
        YB[y0:y0 + n, j * 128:(j + 1) * 128] = y.astype(bf16)
        return y[0:8]

    def post_rows(row0, y0, n, fresh=None, rel=None):
        rows = _ds(row0, n, 16)
        x1 = _rbf(after(X[rows, :], rel).astype(f32) + after(YB[y0:y0 + n, :], rel).astype(f32))
        xb16 = _ln(x1).astype(bf16)
        xb = xb16.astype(f32)
        X[_ds(XBO + row0, n, 16), :] = xb16
        xo = (x1 + xb).astype(bf16)
        X[rows, :] = xo
        r = _rbf(jnp.sum(xb * WR[0:1, :], axis=1, keepdims=True))
        bits = pltpu.bitcast(jnp.broadcast_to(r, (n, 128)), i32)
        key = bits ^ ((bits >> 31) & 0x7FFF0000)
        key = key | (S - 1 - row0 - lax.broadcasted_iota(i32, (n, 128), 0))
        t1 = TOP[0:8, :]
        t2 = TOP[8:16, :]
        for j in range(n // 8):
            kj = key[j * 8:(j + 1) * 8]
            t2 = jnp.maximum(t2, jnp.minimum(t1, kj))
            t1 = jnp.maximum(t1, kj)
        if fresh is not None:
            t1 = jnp.where(fresh, IMIN, t1)
            t2 = jnp.where(fresh, IMIN, t2)
        TOP[0:8, :] = t1
        TOP[8:16, :] = t2
        return done(xo, t2)

    def ln_a(dst_ref, src, dst, n, rel=None):
        y = _ln(after(X[_ds(src, n, 16), :], rel).astype(f32)).astype(bf16)
        dst_ref[_ds(dst, n, 16), :] = y
        return done(y)

    def group_iter(s, g, slot, first_seg, nxt, tail=False):
        par = s % 2
        r0 = g * CH
        mem = not first_seg
        last = nxt is None
        if last:
            P = lambda kind, c, *pins, **kw: None
        else:
            def P(kind, c, *pins, extra=()):
                gate = None
                if pins:
                    v = pins[0]
                    for w in pins[1:]:
                        v = v + w
                    gate = pltpu.bitcast(jnp.minimum(v, 0.0), u32)
                for e in extra:
                    if e is not None:
                        gate = e if gate is None else gate | e
                return proj_part(kind, c, nxt[0], nxt[1], 1 - slot, gate)
        if mem:
            row0 = (s - 1) * L + r0
            if isinstance(row0, int):
                prow, fresh = row0 - CH, None
            else:
                fresh = row0 == 0
                prow = jnp.where(fresh, S, row0 - CH)
        fg = flush(par, g) if slot == 0 else (None, None)
        lsrc = ((s + 1) * L + r0 + 2 * CH) % S

        def LN(t, rel):
            return None if tail else ln_a(LS, lsrc + t, slot * CH + t, SB, None if rel is None else done(rel))

        if mem:
            mem_update(par, g)
        hist = []

        def E(i, h, ms, rel, off=0):
            return expo(i, h, ms, hist, None if rel is None else rel[off:])

        if last:
            m3 = qk(3, slot)
            l3 = [E(3, h, m3, None) for h in range(HG)]
            m2 = qk(2, slot)
            m0 = qk(0, slot)
            m1 = qk(1, slot)
            base = s * L
            yb = 2 * CH
            blk = lambda r, n: [(base + r + t, yb + r + t) for t in range(0, n, SB)]
            plan = [(None, CH, [(prow + t, (1 - slot) * CH + t) for t in (0, SB)], (4, 7)),
                    (3 * QB, QB, [(row0 + t, slot * CH + t) for t in (0, SB)], (4, 7)),
                    (2 * QB, QB, blk(3 * QB, QB), (3, 4, 6, 7)),
                    (0, QB, blk(2 * QB, QB), (3, 4, 6, 7)),
                    (QB, 64, blk(0, 96), (5, 6, 7)),
                    (QB + 64, 32, blk(96, 32), (4,)),
                    (QB + 96, 32, blk(QB, 64), (3, 7))]
            for w, (ra0, n, work, due) in enumerate(plan):
                res = []
                for j in range(G):
                    gate = None
                    if j in due:
                        item = work[due.index(j)]
                        back = 3 if n == QB else 4
                        rel = done(res[j - back]) if j >= back and n >= 64 else None
                        gate = post_rows(item[0], item[1], SB, None, rel)
                    if w == 0:
                        res.append(wo_part(j, 1 - par, r0, slot * CH, CH, gate))
                    else:
                        res.append(wo_part(j, par, ra0, yb + ra0, n, gate, slot))
                    if w == 0 and j == 3:
                        pv(3, l3, mem, par, g, slot)
                        l2 = [E(2, h, m2, None) for h in range(HG)]
                        l0 = [E(0, h, m0, None) for h in range(HG)]
                        l1 = [E(1, h, m1, None) for h in range(HG)]
                    if w == 1 and j == 2:
                        pv(2, l2, mem, par, g, slot)
                    if w == 1 and j == 4:
                        pv(0, l0, mem, par, g, slot)
                        pv(1, l1, mem, par, g, slot)
            for item in blk(QB + 64, 64):
                post_rows(item[0], item[1], SB)
            return

        m3 = qk(3, slot, fg[0])
        lg0 = LN(0, m3[HG] if slot else None)
        lg1 = LN(SB, m3[HG + 4])
        ra = P('k', 0)
        l3 = [E(3, 0, m3, None)]
        rb = P('k', 1, extra=[lg0])
        l3.append(E(3, 1, m3, ra))
        ra = P('k', 2, l3[0], extra=[lg1])
        m2 = qk(2, slot)
        l3.append(E(3, 2, m3, rb))
        rb = P('k', 3, l3[1], extra=[fg[1]])
        m0 = qk(0, slot)
        m1 = qk(1, slot)
        l3.append(E(3, 3, m3, ra))
        ra = P('q', 3, l3[2])
        l2 = [E(2, 0, m2, rb)]
        l0 = [E(0, 0, m0, rb, 12)]
        rb = P('v', 0, l3[3])
        o3 = pv(3, l3, mem, par, g, slot)
        vd = [rb[16]]
        for h in range(1, HG):
            l2.append(E(2, h, m2, ra))
            l0.append(E(0, h, m0, ra, 12))
            ra, rb = rb, P('v', h, l2[h - 1], l0[h - 1], extra=[o3, vd[0]] if h == 3 else [])
            vd.append(rb[16])
        l1 = [E(1, h, m1, ra, 8 * h) for h in range(2)]
        ra = P('q', 2, l2[3], l0[3], extra=[vd[1]])
        o2 = pv(2, l2, mem, par, g, slot)
        o0 = pv(0, l0, mem, par, g, slot)
        l1 += [E(1, h, m1, rb, 8 * (h - 2)) for h in range(2, 4)]
        ra = P('q', 1, *l1, extra=[vd[2]])
        o1 = pv(1, l1, mem, par, g, slot)
        if not mem:
            P('q', 0, extra=[vd[3]])
            return
        rb = P('q', 0, extra=[vd[3]])
        gates = {1: o2 | o0, 4: o1}
        gates[3] = post_rows(prow, (1 - slot) * CH, SB, fresh, done(ra[0]))
        gates[7] = post_rows(prow + SB, (1 - slot) * CH + SB, SB, fresh, done(rb[8]))
        for j in range(G):
            wo_part(j, 1 - par, r0, slot * CH, CH, gates.get(j))

    def ffn():
        t = TOP[...]
        k1 = jnp.max(t, axis=0, keepdims=True)
        k2 = jnp.max(jnp.where(t == k1, IMIN, t), axis=0, keepdims=True)
        sub = lax.broadcasted_iota(i32, (16, D), 0)
        idx, blks, sgs = [], [], []
        for kk in (k1, k2):
            ii = jnp.clip(S - 1 - (jnp.max(kk) & 0xFFFF), 0, S - 1)
            hi = kk & (-65536)
            rv = pltpu.bitcast(hi ^ ((hi >> 31) & 0x7FFF0000), f32)
            sgs.append(_rbf(_sigmoid(rv))[:, 0:1])
            idx.append(ii)
            blks.append(X[pl.ds(pl.multiple_of(XBO + ((ii >> 4) << 4), 16), 16), :])
        xs = jnp.concatenate(blks, axis=0)
        gt = _rbf(_dot(xs, WG[...]))
        up = _rbf(_dot(xs, WU[...]))
        hh = (_rbf(gt * _sigmoid(gt)) * up).astype(bf16)
        nk = 4
        kc = F // nk
        y = _dot(hh[:, 0:kc], WD[0:kc, :])
        for j in range(1, nk):
            y = y + _dot(hh[:, j * kc:(j + 1) * kc], WD[j * kc:(j + 1) * kc, :])
        y = _rbf(y)
        return idx, [_rbf(y[j * 16:(j + 1) * 16, :] * sgs[j]) for j in range(2)], sub

    def patch(idx, ys, sub):
        for ii, yj in zip(idx, ys):
            b = pl.multiple_of((ii >> 4) << 4, 16)
            blk = X[pl.ds(b, 16), :].astype(f32)
            X[pl.ds(b, 16), :] = jnp.where(sub == (ii & 15), blk + yj, blk).astype(bf16)

    def layer_body(layer, carry):
        MEM[...] = jnp.zeros(MEM.shape, f32)
        TOP[...] = jnp.full(TOP.shape, IMIN, i32)
        lg = [ln_a(LS, L + t, t, CH) for t in (0, CH)]
        for kind in 'vkq':
            for c in range(4):
                proj_part(kind, c, 0, 0, 0, lg[c // 2] if (kind == 'k' and c % 2 == 1) else None)

        @pl.when(layer == 0)
        def _():
            x_copy(1).wait()

        def body_a(j, c):
            @pl.when(layer == 0)
            def _():
                for u in range(U):
                    g = j * U + u + 1

                    @pl.when(g < G)
                    def _():
                        for cp in w_copies(g):
                            cp.wait()

                    @pl.when(g + U < G)
                    def _():
                        for cp in w_copies(g + U):
                            cp.start()

                @pl.when(j == 1)
                def _():
                    wo_copy.start()
                    x_copy(2).start()
                    x_copy(3).start()

                @pl.when(j == G // U - 1)
                def _():
                    x_copy(2).wait()

            for u in range(U):
                g = j * U + u
                if u < U - 1:
                    nxt = (0, g + 1)
                else:
                    nxt = (jnp.where(j == G // U - 1, 1, 0), (g + 1) % G)
                group_iter(0, g, u % 2, True, nxt)
            return c

        lax.fori_loop(0, G // U, body_a, 0)

        @pl.when(layer == 0)
        def _():
            wo_copy.wait()
            x_copy(3).wait()
            wg_copy.start()
            wu_copy.start()
            wd_copy.start()

        def body_b(it, c):
            s = 1 + it // (G // U)
            j = it % (G // U)
            for u in range(U):
                g = j * U + u
                if u < U - 1:
                    nxt = (s % 2, g + 1)
                else:
                    nxt = ((s + jnp.where(j == G // U - 1, 1, 0)) % 2, (g + 1) % G)
                group_iter(s, g, u % 2, False, nxt)

            @pl.when(jnp.logical_and(layer == 1, jnp.logical_and(j == 0, s >= 2)))
            def _():
                out_copy(jnp.maximum(s - 2, 0)).start()

            return c

        lax.fori_loop(0, 3 * (G // U) - 1, body_b, 0)
        s = NSEG - 1
        for g in range(G - U, G):
            group_iter(s, g, g % 2, False, (s % 2, g + 1) if g < G - 1 else None, tail=True)

        @pl.when(layer == 0)
        def _():
            wg_copy.wait()
            wu_copy.wait()
            wd_copy.wait()

        @pl.when(layer == 1)
        def _():
            out_copy(NSEG - 2).start()
            out_copy(NSEG - 1).start()

        idx, ys, sub = ffn()

        @pl.when(layer == 1)
        def _():
            for s in range(NSEG):
                out_copy(s).wait()

        patch(idx, ys, sub)

        @pl.when(layer == 0)
        def _():
            for ii in idx:
                @pl.when(ii < L)
                def _():
                    b = (ii >> 4) << 4
                    ln_a(XN, b, b, 16)

        @pl.when(layer == 1)
        def _():
            bs = [pl.multiple_of((ii >> 4) << 4, 16) for ii in idx]
            cps = [pltpu.make_async_copy(X.at[pl.ds(b, 16), :], out_hbm.at[0, pl.ds(b, 16), :], sem_o.at[j])
                   for j, b in enumerate(bs)]
            cps[0].start()

            @pl.when(bs[0] != bs[1])
            def _():
                cps[1].start()
                cps[1].wait()

            cps[0].wait()

        return carry

    lax.fori_loop(0, 2, layer_body, 0)


def _pk(*shape):
    return pltpu.VMEM((*shape[:-2], shape[-2] // 2, shape[-1]), u32)


@jax.jit
def pallas_interleave_layers__memory_aug_infini_attn__moe_arch_mod__prompt_kernel(
    A_x: jax.Array,
    A_wq: jax.Array,
    A_wk: jax.Array,
    A_wv: jax.Array,
    A_wo: jax.Array,
    A_beta: jax.Array,
    B_x: jax.Array,
    B_w_r: jax.Array,
    B_w_gate: jax.Array,
    B_w_up: jax.Array,
    B_w_down: jax.Array,
):
    del B_x
    any_spec = pl.BlockSpec(memory_space=pl.ANY)
    vmem_spec = pl.BlockSpec(memory_space=pltpu.VMEM)
    scratch = [
        _pk(2 * XBO, D),
        _pk(2 * L, D),
        _pk(2 * CH, D),
        _pk(G, D, 384),
        _pk(D, D),
        _pk(D, F),
        _pk(D, F),
        _pk(F, D),
        _pk(2 * L, 256),
        _pk(2 * L, 256),
        _pk(2 * L, 256),
        _pk(2 * 128, L),
        _pk(2 * G * L, 256),
        _pk(2 * G * MR, L),
        _pk(2 * G * L + 16, 256),
        _pk(MR, 256),
        _pk(QB, 512), _pk(2 * QB, 512), _pk(3 * QB, 512), _pk(4 * QB, 512),
        _pk(2 * CH + L, D),
        _pk(2 * QB, 256), _pk(2 * QB, 256), _pk(2 * QB, 256), _pk(2 * QB, 256),
        pltpu.VMEM((QB, 512), f32), pltpu.VMEM((2 * QB, 512), f32),
        pltpu.VMEM((3 * QB, 512), f32), pltpu.VMEM((4 * QB, 512), f32),
        pltpu.VMEM((G, MR, 128), f32),
        pltpu.VMEM((16, 128), i32),
        pltpu.VMEM((H, 128), f32),
        pltpu.VMEM((128, 128), f32),
        pltpu.VMEM((MR, 128), f32),
        pltpu.VMEM((8, D), f32),
        pltpu.SMEM((8,), i32),
        pltpu.SemaphoreType.DMA((NSEG + 5,)),
        pltpu.SemaphoreType.DMA((3 * G + 1,)),
        pltpu.SemaphoreType.DMA((3,)),
        pltpu.SemaphoreType.DMA((NSEG,)),
    ]
    return pl.pallas_call(
        _kernel,
        out_shape=jax.ShapeDtypeStruct((1, S, D), bf16),
        in_specs=[any_spec, any_spec, any_spec, any_spec, any_spec, vmem_spec, vmem_spec,
                  any_spec, any_spec, any_spec],
        out_specs=any_spec,
        scratch_shapes=scratch,
        compiler_params=pltpu.CompilerParams(vmem_limit_bytes=100 * 2 ** 20),
    )(A_x, A_wq, A_wk, A_wv, A_wo, A_beta.reshape(1, H), B_w_r.reshape(1, D), B_w_gate, B_w_up, B_w_down)
```

```python
import functools
import math

import jax
import jax.numpy as jnp
from jax import lax
import jax.experimental.pallas as pl
import jax.experimental.pallas.tpu as pltpu

S = 2048
D = 1024
H = 32
DH = 32
NSEG = 4
L = S // NSEG
F = 3584
G = 8
HG = 4
QB = 128
NQB = L // QB
MR = 144
CH = L // G
U = 2
SB = 32
PD = 16
PE = 4
XBO = S + CH
EPS = 1e-5
LOG2E = math.log2(math.e)
QSCALE = (DH ** -0.5) * LOG2E
NEG = -1e9 * LOG2E
IMIN = -2 ** 31

f32 = jnp.float32
bf16 = jnp.bfloat16
i32 = jnp.int32
u32 = jnp.uint32

NT = (((1,), (1,)), ((), ()))


def _rbf(x):
    return x.astype(bf16).astype(f32)


def _recip(x):
    r = pl.reciprocal(x, approx=True)
    return r * (2.0 - x * r)


def _rstd(v):
    a = _rbf(_rbf(v) + EPS)
    y = lax.rsqrt(a)
    sd = _rbf(a * y)
    return y * (2.0 - sd * y)


def _ln(x):
    m = jnp.sum(x, axis=1, keepdims=True) * (1.0 / D)
    mb = _rbf(m)
    c = x - mb
    e = m - mb
    return c * _rstd(jnp.maximum(jnp.sum(c * c, axis=1, keepdims=True) * (1.0 / D) - e * e, 0.0))


def _stats(xs):
    p = jnp.broadcast_to(xs[0][:, 0:1], xs[0].shape)
    s = q = None
    for xc in xs:
        d = xc - p
        s = d if s is None else s + d
        q = d * d if q is None else q + d * d
    sm = jnp.sum(s, axis=1, keepdims=True) * (1.0 / D)
    v = jnp.sum(q, axis=1, keepdims=True) * (1.0 / D) - sm * sm
    return _rbf(p + sm), _rstd(v)


def _phi(t):
    return jnp.where(t > 0, t + 1.0, jnp.exp(t))


def _sigmoid(t):
    return 1.0 / (1.0 + jnp.exp(-t))


def _dot(a, b):
    return jnp.dot(a, b, preferred_element_type=f32)


def _dot_nt(a, b):
    return lax.dot_general(a, b, NT, preferred_element_type=f32)


def _ds(start, size, mult):
    if isinstance(start, int):
        return pl.ds(start, size)
    return pl.ds(pl.multiple_of(start, mult), size)


def _colred(p, op, nacc=2):
    n = p.shape[0]
    parts = [p[j * 8:(j + 1) * 8] for j in range(n // 8)]
    acc = parts[:nacc]
    for j in range(nacc, len(parts)):
        acc[j % nacc] = op(acc[j % nacc], parts[j])
    r = acc[0]
    for a in acc[1:]:
        r = op(r, a)
    return r


def _kernel(x_hbm, wq_hbm, wk_hbm, wv_hbm, wo_hbm, beta_ref, wr_ref, wg_hbm, wu_hbm, wd_hbm,
            out_hbm,
            X, XN, LS, W3, WO, WG, WU, WD,
            KB, QS, PQ, VT, PKS, VTS, OB, MEMB, PB0, PB1, PB2, PB3, YB, OS0, OS1, OS2, OS3, XS0, XS1, ST0, ST1,
            SC0, SC1, SC2, SC3, MEM, TOP, GATE, MASK, MMASK, WR, ZS,
            sem_x, sem_w, sem_f, sem_o):
    X, XN, LS, W3, WO, WG, WU, WD, KB, QS, PQ, VT, PKS, VTS, OB, MEMB, YB = [
        r.bitcast(bf16) for r in
        (X, XN, LS, W3, WO, WG, WU, WD, KB, QS, PQ, VT, PKS, VTS, OB, MEMB, YB)]
    PB = [r.bitcast(bf16) for r in (PB0, PB1, PB2, PB3)]
    OS = [r.bitcast(bf16) for r in (OS0, OS1, OS2, OS3)]
    XS = [r.bitcast(bf16) for r in (XS0, XS1)]
    ST = (ST0, ST1)
    SC = (SC0, SC1, SC2, SC3)

    def x0_copy(c):
        return pltpu.make_async_copy(x_hbm.at[0, pl.ds(c * 128, 128), :], X.at[pl.ds(c * 128, 128), :],
                                     sem_x.at[NSEG + c])

    def x_copy(s):
        r0 = s * L + (128 if s == 1 else 0)
        n = (s + 1) * L - r0
        return pltpu.make_async_copy(x_hbm.at[0, pl.ds(r0, n), :], X.at[pl.ds(r0, n), :], sem_x.at[s])

    def w_copies(g):
        col = pl.multiple_of(g * 128, 128)
        return [pltpu.make_async_copy(w.at[:, pl.ds(col, 128)], W3.at[g, :, pl.ds(j * 128, 128)],
                                      sem_w.at[3 * g + j])
                for j, w in enumerate((wk_hbm, wq_hbm, wv_hbm))]

    wo_copy = pltpu.make_async_copy(wo_hbm, WO, sem_w.at[3 * G])
    wg_copy = pltpu.make_async_copy(wg_hbm, WG, sem_f.at[0])
    wu_copy = pltpu.make_async_copy(wu_hbm, WU, sem_f.at[1])
    wd_copy = pltpu.make_async_copy(wd_hbm, WD, sem_f.at[2])

    def out_copy(s):
        base = pl.multiple_of(s * L, L)
        return pltpu.make_async_copy(X.at[pl.ds(base, L), :], out_hbm.at[0, pl.ds(base, L), :], sem_o.at[s])

    x0_copy(0).start()
    for cp in w_copies(0):
        cp.start()
    for c in range(1, 5):
        x0_copy(c).start()
    for g in range(1, 1 + U):
        for cp in w_copies(g):
            cp.start()
    x_copy(1).start()

    row = lax.broadcasted_iota(i32, (128, 128), 0)
    col = lax.broadcasted_iota(i32, (128, 128), 1)
    MASK[...] = jnp.where(row > col, NEG, 0.0).astype(f32)
    r144 = lax.broadcasted_iota(i32, (MR, 128), 0)
    c144 = lax.broadcasted_iota(i32, (MR, 128), 1)
    head_of_row = jnp.where(r144 < 128, r144 >> 5, r144 - 128)
    MMASK[...] = jnp.where(head_of_row == (c144 >> 5), 1.0, 0.0).astype(f32)
    for t in range(2 * G):
        VTS[t * MR + 128:(t + 1) * MR, :] = jnp.ones((MR - 128, L), bf16)
    for j in range(8):
        ZS[j] = 0
    X[S:S + CH, :] = jnp.zeros((CH, D), bf16)
    for r in OS:
        r[:, 0:128] = jnp.zeros((2 * QB, 128), bf16)
    OB[2 * G * L:2 * G * L + 16, 0:128] = jnp.zeros((16, 128), bf16)
    YB[CH:2 * CH, :] = jnp.zeros((CH, D), bf16)
    gsig = _rbf(_sigmoid(beta_ref[...].astype(f32)))
    r32 = lax.broadcasted_iota(i32, (H, H), 0)
    c32 = lax.broadcasted_iota(i32, (H, H), 1)
    gcol = jnp.sum(jnp.where(r32 == c32, jnp.broadcast_to(gsig, (H, H)), 0.0), axis=1, keepdims=True)
    GATE[...] = jnp.broadcast_to(gcol, (H, 128))
    WR[...] = jnp.broadcast_to(wr_ref[...].astype(f32), (8, D))

    lane128 = lax.broadcasted_iota(i32, (QB // 2, 128), 1) >> 5

    def gated(x, gate, slots=None):
        if gate is None and not slots:
            return x
        xu = pltpu.bitcast(x, u32)
        slots = dict(slots or {})
        if gate is not None:
            for t in range(4):
                slots[(t, 0)] = gate if (t, 0) not in slots else slots[(t, 0)] | gate
        rows = []
        for b in range(xu.shape[0] // 8):
            blk = xu[b * 8:(b + 1) * 8]
            if any(k[1] == b for k in slots):
                blk = jnp.concatenate(
                    [blk[:, t * 128:(t + 1) * 128] | slots[(t, b)] if (t, b) in slots else blk[:, t * 128:(t + 1) * 128]
                     for t in range(xu.shape[1] // 128)], axis=1)
            rows.append(blk)
        return pltpu.bitcast(jnp.concatenate(rows, axis=0), bf16)

    def spread(gates, nb, first=0):
        return {(4 * (i // nb) + i % 4, i % nb): gt for i, gt in enumerate(gates, first)}

    def done(*vals):
        acc = None
        for v in vals:
            w = pltpu.bitcast(v, u32)
            for r in range(0, w.shape[0], 8):
                for c in range(0, w.shape[1], 128):
                    t = w[r:r + 8, c:c + 128]
                    acc = t if acc is None else acc | t
        return acc & jnp.full((8, 128), ZS[3], i32).astype(u32)

    def after(x, gate):
        if gate is None:
            return x
        xu = pltpu.bitcast(x, u32)
        return pltpu.bitcast(xu | jnp.tile(gate, (xu.shape[0] // 8, xu.shape[1] // 128)), bf16)

    def proj_part(kind, c, par, g, slot, gate=None, slots=None):
        rows = slice(c * 128, (c + 1) * 128)
        srows = slice(slot * L + c * 128, slot * L + (c + 1) * 128)
        item = par * G + g
        j = 'kqv'.index(kind)
        x = XN[_ds(par * L + c * 128 + ZS[j], 128, 128), :]
        x = gated(x, gate, slots)
        r = _dot(x, W3[g, :, j * 128:(j + 1) * 128])
        if kind == 'v':
            vt = r.astype(bf16).T
            VT[slot * 128:(slot + 1) * 128, rows] = vt
            VTS[_ds(item * MR, 128, 16), rows] = vt
            return [jnp.abs(r[t * 8:(t + 1) * 8]) for t in range(16)] + [done(vt)]
        ph = _phi(r)
        if kind == 'k':
            KB[srows, 0:128] = r.astype(bf16)
            PKS[_ds(item * L + c * 128, 128, 128), 0:128] = ph.astype(bf16)
        else:
            QS[srows, 0:128] = (r * QSCALE).astype(bf16)
            PQ[srows, 0:128] = ph.astype(bf16)
        return [ph[t * 8:(t + 1) * 8] for t in range(16)]

    def mem_update(par, g):
        prev = (1 - par) * G + g
        m = MEM[g] + _dot(VTS[_ds(prev * MR, MR, 16), :], PKS[_ds(prev * L, L, L), 0:128])
        MEM[g] = m
        MEMB[:, 0:128] = (m * MMASK[...]).astype(bf16)

    def qk(i, slot, gate=None):
        n = QB * (i + 1)
        qi = pltpu.bitcast(QS[slot * L + i * QB:slot * L + (i + 1) * QB, 0:128], u32)
        qm = jnp.concatenate(
            [pltpu.bitcast(jnp.where(lane128 == h, qi, jnp.uint32(0)), bf16) for h in range(HG)], axis=0)
        kb = KB[slot * L:slot * L + n, 0:128]
        if gate is not None:
            kb = jnp.concatenate([after(kb[0:16], gate), kb[16:]], axis=0)
        st = _dot_nt(kb, qm)
        ms = []
        for h in range(HG):
            sh = st[:, h * QB:(h + 1) * QB]
            sd = sh[n - QB:, :] + MASK[...]
            sh = sd if i == 0 else jnp.concatenate([sh[:n - QB, :], sd], axis=0)
            SC[i][:, h * QB:(h + 1) * QB] = sh
            ms.append(jnp.max(_colred(sh, jnp.maximum), axis=0, keepdims=True))
        return ms + [st[t:t + 8, 0:QB] for t in range(0, n, 16)]

    def expo(i, h, ms, hist, rel):
        n = QB * (i + 1)
        z = ZS[0]
        sc = SC[i][_ds(z, n, 8), h * QB:(h + 1) * QB]
        m = jnp.broadcast_to(ms[h], (8, QB))
        ps = []
        acc = [None, None]
        for k in range(n // 8):
            if k % PE == 0:
                pace = rel[k // PE] if rel is not None else (hist[-PD] if len(hist) >= PD else None)
                mk = m if pace is None else m + jnp.minimum(pace, 0.0)
            pk = jnp.exp2(sc[k * 8:(k + 1) * 8] - mk)
            acc[k % 2] = pk if acc[k % 2] is None else acc[k % 2] + pk
            hist.append(acc[k % 2])
            ps.append(pk)
        PB[i][:, h * QB:(h + 1) * QB] = jnp.concatenate(ps, axis=0).astype(bf16)
        return acc[0] + acc[1]

    def pv(i, ls, use_mem, par, g, slot):
        n = QB * (i + 1)
        if use_mem:
            mrd = _dot_nt(MEMB[:, 0:128], PQ[slot * L + i * QB:slot * L + (i + 1) * QB, 0:128])
        outs = []
        z = ZS[0]
        for h in range(HG):
            o = _dot(VT[slot * 128 + h * DH:slot * 128 + (h + 1) * DH, 0:n], PB[i][_ds(z, n, 16), h * QB:(h + 1) * QB])
            gt = GATE[pl.ds(g * HG + h, 1), :]
            o = o * ((1.0 - gt) * _recip(jnp.sum(ls[h], axis=0, keepdims=True)))
            if use_mem:
                num = mrd[h * DH:(h + 1) * DH, :]
                den = mrd[128 + h:129 + h, :] + 1e-6
                o = num * (gt * _recip(den)) + o
            outs.append(o)
        ot = jnp.concatenate(outs, axis=0)
        ot = ot.astype(bf16).T
        OS[i][slot * QB:(slot + 1) * QB, 0:128] = ot
        return done(ot)

    def flush(par, g):
        XN[_ds((1 - par) * L + g * CH, 2 * CH, 2 * CH), :] = LS[...]
        g1 = done(XN[_ds(ZS[4], 16, 16), 0:128])
        prev = (par * G + g + 2 * G - 2) % (2 * G)
        for u in range(2):
            for i in range(NQB):
                OB[_ds((prev + u) * L + i * QB, QB, QB), 0:128] = OS[i][u * QB:(u + 1) * QB, 0:128]
        return g1, done(OB[_ds(2 * G * L + ZS[4], 16, 16), 0:128])

    def wo_part(j, par, r0, y0, n, gate=None, live=None, slots=None):
        o = [OB[_ds((par * G + g) * L + r0 + ZS[j], n, 16), 0:128] for g in range(G if live is None else G - 2)]
        if live is not None:
            o += [OS[r0 // QB][_ds(u * QB + r0 % QB + ZS[j], n, 16), 0:128] for u in range(2)]
        o = jnp.concatenate(o, axis=1)
        y = _dot(gated(o, gate, slots), WO[:, j * 128:(j + 1) * 128])
        YB[y0:y0 + n, j * 128:(j + 1) * 128] = y.astype(bf16)
        return [y[t:t + 8] for t in range(0, n, 16)]

    def chunks(ref, rows, rel, skip=0):
        out = []
        for c in range(D // 128):
            gate = None if (rel is None or c < skip) else rel[c * len(rel) // 8]
            out.append(after(ref[rows, c * 128:(c + 1) * 128], gate).astype(f32))
        return out

    def post1(row0, y0, n, xs, rel=None, park=False):
        x = chunks(X, _ds(row0, n, 16), rel, 1)
        y = chunks(YB, slice(y0, y0 + n), rel, 1)
        x1 = [(a + b).astype(bf16) for a, b in zip(x, y)]
        XS[xs][...] = jnp.concatenate(x1, axis=1)
        st = _stats([a.astype(f32) for a in x1])
        if park:
            st = (st[0], jnp.broadcast_to(st[1], (n, 128)))
            ST[xs][0:n, :] = st[0]
            ST[xs][n:2 * n, :] = st[1]
        else:
            st = (st[0] + jnp.minimum(st[1], 0.0), st[1])
        return st, [done(a) for a in x1]

    def post2(row0, n, xs, st, cs, rel=None, r=None):
        mb, rs = st
        out = []
        for i, c in enumerate(cs):
            cols = slice(c * 128, (c + 1) * 128)
            x1 = after(XS[xs][_ds(ZS[5], n, 16), cols], None if rel is None else rel[i]).astype(f32)
            xb16 = ((x1 - mb) * rs).astype(bf16)
            xb = xb16.astype(f32)
            X[_ds(XBO + row0, n, 16), cols] = xb16
            xo = (x1 + xb).astype(bf16)
            X[_ds(row0, n, 16), cols] = xo
            out.append(done(xo))
            t = xb * WR[0:1, cols]
            r = t if r is None else r + t
        return r, out

    def post3(row0, n, r, fresh=None):
        r = _rbf(jnp.sum(r, axis=1, keepdims=True))
        bits = pltpu.bitcast(jnp.broadcast_to(r, (n, 128)), i32)
        key = bits ^ ((bits >> 31) & 0x7FFF0000)
        key = key | (S - 1 - row0 - lax.broadcasted_iota(i32, (n, 128), 0))
        t1 = TOP[0:8, :]
        t2 = TOP[8:16, :]
        for j in range(n // 8):
            kj = key[j * 8:(j + 1) * 8]
            t2 = jnp.maximum(t2, jnp.minimum(t1, kj))
            t1 = jnp.maximum(t1, kj)
        if fresh is not None:
            t1 = jnp.where(fresh, IMIN, t1)
            t2 = jnp.where(fresh, IMIN, t2)
        TOP[0:8, :] = t1
        TOP[8:16, :] = t2
        return done(t2)

    cnt = [0]

    def post_rows(row0, y0, n, fresh=None, rel=None):
        cnt[0] += 1
        xs = cnt[0] % 2
        r, xo = post2(row0, n, xs, post1(row0, y0, n, xs, None if rel is None else [rel])[0], range(8))
        return functools.reduce(lambda a, b: a | b, xo, post3(row0, n, r, fresh))

    def ln_a(dst_ref, src, dst, n, rel=None, rel2=None):
        mb, rs = _stats(chunks(X, _ds(src, n, 16), rel, 1))
        mb = mb + jnp.minimum(rs, 0.0)
        y = [((a - mb) * rs).astype(bf16) for a in chunks(X, _ds(src + ZS[5], n, 16), rel2)]
        dst_ref[_ds(dst, n, 16), :] = jnp.concatenate(y, axis=1)
        return [done(a) for a in y]

    def group_iter(s, g, slot, first_seg, nxt, tail=False):
        par = s % 2
        r0 = g * CH
        mem = not first_seg
        last = nxt is None
        if last:
            P = lambda kind, c, *pins, **kw: None
        else:
            def P(kind, c, *pins, extra=(), slots=None):
                gate = None
                if pins:
                    v = pins[0]
                    for w in pins[1:]:
                        v = v + w
                    gate = pltpu.bitcast(jnp.minimum(v, 0.0), u32)
                for e in extra:
                    if e is not None:
                        gate = e if gate is None else gate | e
                return proj_part(kind, c, nxt[0], nxt[1], 1 - slot, gate, slots)
        if mem:
            row0 = (s - 1) * L + r0
            if isinstance(row0, int):
                prow, fresh = row0 - CH, None
            else:
                fresh = row0 == 0
                prow = jnp.where(fresh, S, row0 - CH)
        fg = flush(par, g) if slot == 0 else (None, None)
        lsrc = ((s + 1) * L + r0 + 2 * CH) % S

        dn = lambda vs: [done(v) for v in vs]

        def LN(t, rel, rel2):
            return [] if tail else ln_a(LS, lsrc + t, slot * CH + t, SB, None if rel is None else dn(rel), dn(rel2))

        if mem:
            mem_update(par, g)
        hist = []

        def E(i, h, ms, rel, off=0):
            return expo(i, h, ms, hist, None if rel is None else rel[off:])

        if last:
            m3 = qk(3, slot)
            l3 = [E(3, h, m3, None) for h in range(HG)]
            m2 = qk(2, slot)
            m0 = qk(0, slot)
            m1 = qk(1, slot)
            base = s * L
            yb = 2 * CH
            blk = lambda r, n: [(base + r + t, yb + r + t) for t in range(0, n, SB)]
            plan = [(None, CH, [(prow + t, (1 - slot) * CH + t) for t in (0, SB)], (4, 7)),
                    (3 * QB, QB, [(row0 + t, slot * CH + t) for t in (0, SB)], (4, 7)),
                    (2 * QB, QB, blk(3 * QB, QB), (3, 4, 6, 7)),
                    (0, QB, blk(2 * QB, QB), (3, 4, 6, 7)),
                    (QB, 64, blk(0, 96), (5, 6, 7)),
                    (QB + 64, 32, blk(96, 32), (4,)),
                    (QB + 96, 32, blk(QB, 64), (3, 7))]
            for w, (ra0, n, work, due) in enumerate(plan):
                res = []
                for j in range(G):
                    gate = None
                    if j in due:
                        item = work[due.index(j)]
                        back = 3 if n == QB else 4
                        rel = done(res[j - back][0]) if j >= back and n >= 64 else None
                        gate = post_rows(item[0], item[1], SB, None, rel)
                    if w == 0:
                        res.append(wo_part(j, 1 - par, r0, slot * CH, CH, gate))
                    else:
                        res.append(wo_part(j, par, ra0, yb + ra0, n, gate, slot))
                    if w == 0 and j == 3:
                        pv(3, l3, mem, par, g, slot)
                        l2 = [E(2, h, m2, None) for h in range(HG)]
                        l0 = [E(0, h, m0, None) for h in range(HG)]
                        l1 = [E(1, h, m1, None) for h in range(HG)]
                    if w == 1 and j == 2:
                        pv(2, l2, mem, par, g, slot)
                    if w == 1 and j == 4:
                        pv(0, l0, mem, par, g, slot)
                        pv(1, l1, mem, par, g, slot)
            for item in blk(QB + 64, 64):
                post_rows(item[0], item[1], SB)
            return

        m3 = qk(3, slot, fg[0])
        lg0 = LN(0, m3[HG:HG + 8] if slot else None, m3[HG + 20:HG + 28])
        lg1 = LN(SB, m3[HG + 8:HG + 16], m3[HG + 28:HG + 32])
        ra = P('k', 0, slots=spread(lg0, 8, 8))
        l3 = [E(3, 0, m3, None)]
        rb = P('k', 1, slots=spread(lg1, 8))
        l3.append(E(3, 1, m3, ra))
        ra = P('k', 2, l3[0])
        m2 = qk(2, slot)
        l3.append(E(3, 2, m3, rb))
        two = lambda gs: {k: v for i, gt in enumerate(gs) for k, v in spread([gt], 8, 2 * i).items()}
        if mem:
            sa, da = post1(prow, (1 - slot) * CH, SB, 0, dn(m2[HG::3]), True)
        rb = P('k', 3, l3[1], extra=[fg[1]], slots=two(da) if mem else None)
        m0 = qk(0, slot)
        m1 = qk(1, slot)
        l3.append(E(3, 3, m3, ra))
        if mem:
            sb, db = post1(prow + SB, (1 - slot) * CH + SB, SB, 1, dn((m0[HG:] + m1[HG:])[::3]), True)
        ra = P('q', 3, l3[2], extra=[done(*sa)] if mem else [], slots=two(db) if mem else None)
        l2 = [E(2, 0, m2, rb)]
        l0 = [E(0, 0, m0, rb, 12)]
        rb = P('v', 0, l3[3])
        o3 = pv(3, l3, mem, par, g, slot)
        vd = [rb[16]]
        for h in range(1, HG):
            l2.append(E(2, h, m2, ra))
            l0.append(E(0, h, m0, ra, 12))
            ra, rb = rb, P('v', h, l2[h - 1], l0[h - 1], extra=[o3, vd[0]] if h == 3 else [done(*sb)] if h == 1 and mem else [])
            vd.append(rb[16])
        l1 = [E(1, h, m1, ra, 8 * h) for h in range(2)]
        ra = P('q', 2, l2[3], l0[3], extra=[vd[1]])
        o2 = pv(2, l2, mem, par, g, slot)
        o0 = pv(0, l0, mem, par, g, slot)
        l1 += [E(1, h, m1, rb, 8 * (h - 2)) for h in range(2, 4)]
        ra = P('q', 1, *l1, extra=[vd[2]])
        o1 = pv(1, l1, mem, par, g, slot)
        if not mem:
            P('q', 0, extra=[vd[3]])
            return
        P('q', 0, extra=[vd[3]])
        gates = {1: o2 | o0, 4: o1}
        slots = {}
        sa, sb = [(ST[i][_ds(ZS[5], SB, 8), :], ST[i][_ds(SB + ZS[5], SB, 8), :]) for i in range(2)]
        r = None
        for j in range(G):
            res = wo_part(j, 1 - par, r0, slot * CH, CH, gates.get(j), None, slots.get(j))
            if j < 4:
                row = prow + SB * (j // 2)
                r, e = post2(row, SB, j // 2, sb if j // 2 else sa, range(4 * (j % 2), 4 * (j % 2) + 4), dn(res), r)
                slots[j + 2] = spread(e, 4, 4)
                if j == 1:
                    gates[6] = post3(row, SB, r, fresh)
                    r = None
                if j == 3:
                    t = post3(row, SB, r, fresh)
                    slots[7] = {(4 + i, 0): t for i in range(4)}

    def ffn():
        t = TOP[...]
        k1 = jnp.max(t, axis=0, keepdims=True)
        k2 = jnp.max(jnp.where(t == k1, IMIN, t), axis=0, keepdims=True)
        sub = lax.broadcasted_iota(i32, (16, D), 0)
        idx, blks, sgs = [], [], []
        for kk in (k1, k2):
            ii = jnp.clip(S - 1 - (jnp.max(kk) & 0xFFFF), 0, S - 1)
            hi = kk & (-65536)
            rv = pltpu.bitcast(hi ^ ((hi >> 31) & 0x7FFF0000), f32)
            sgs.append(_rbf(_sigmoid(rv))[:, 0:1])
            idx.append(ii)
            blks.append(X[pl.ds(pl.multiple_of(XBO + ((ii >> 4) << 4), 16), 16), :])
        xs = jnp.concatenate(blks, axis=0)
        gt = _rbf(_dot(xs, WG[...]))
        up = _rbf(_dot(xs, WU[...]))
        hh = (_rbf(gt * _sigmoid(gt)) * up).astype(bf16)
        nk = 4
        kc = F // nk
        y = _dot(hh[:, 0:kc], WD[0:kc, :])
        for j in range(1, nk):
            y = y + _dot(hh[:, j * kc:(j + 1) * kc], WD[j * kc:(j + 1) * kc, :])
        y = _rbf(y)
        return idx, [_rbf(y[j * 16:(j + 1) * 16, :] * sgs[j]) for j in range(2)], sub

    def patch(idx, ys, sub):
        for ii, yj in zip(idx, ys):
            b = pl.multiple_of((ii >> 4) << 4, 16)
            blk = X[pl.ds(b, 16), :].astype(f32)
            X[pl.ds(b, 16), :] = jnp.where(sub == (ii & 15), blk + yj, blk).astype(bf16)

    def layer_body(layer, carry):
        MEM[...] = jnp.zeros(MEM.shape, f32)
        TOP[...] = jnp.full(TOP.shape, IMIN, i32)
        lg = [functools.reduce(lambda a, b: a | b, ln_a(LS, L + t, t, CH)) for t in (0, CH)]
        for kind in 'vkq':
            for c in range(4):
                proj_part(kind, c, 0, 0, 0, lg[c // 2] if (kind == 'k' and c % 2 == 1) else None)

        @pl.when(layer == 0)
        def _():
            x_copy(1).wait()

        def body_a(j, c):
            @pl.when(layer == 0)
            def _():
                for u in range(U):
                    g = j * U + u + 1

                    @pl.when(g < G)
                    def _():
                        for cp in w_copies(g):
                            cp.wait()

                    @pl.when(g + U < G)
                    def _():
                        for cp in w_copies(g + U):
                            cp.start()

                @pl.when(j == 1)
                def _():
                    wo_copy.start()
                    x_copy(2).start()
                    x_copy(3).start()

                @pl.when(j == G // U - 1)
                def _():
                    x_copy(2).wait()

            for u in range(U):
                g = j * U + u
                if u < U - 1:
                    nxt = (0, g + 1)
                else:
                    nxt = (jnp.where(j == G // U - 1, 1, 0), (g + 1) % G)
                group_iter(0, g, u % 2, True, nxt)
            return c

        lax.fori_loop(0, G // U, body_a, 0)

        @pl.when(layer == 0)
        def _():
            wo_copy.wait()
            x_copy(3).wait()
            wg_copy.start()
            wu_copy.start()
            wd_copy.start()

        def body_b(it, c):
            s = 1 + it // (G // U)
            j = it % (G // U)
            for u in range(U):
                g = j * U + u
                if u < U - 1:
                    nxt = (s % 2, g + 1)
                else:
                    nxt = ((s + jnp.where(j == G // U - 1, 1, 0)) % 2, (g + 1) % G)
                group_iter(s, g, u % 2, False, nxt)

            @pl.when(jnp.logical_and(layer == 1, jnp.logical_and(j == 0, s >= 2)))
            def _():
                out_copy(jnp.maximum(s - 2, 0)).start()

            return c

        lax.fori_loop(0, 3 * (G // U) - 1, body_b, 0)
        s = NSEG - 1
        for g in range(G - U, G):
            group_iter(s, g, g % 2, False, (s % 2, g + 1) if g < G - 1 else None, tail=True)

        @pl.when(layer == 0)
        def _():
            wg_copy.wait()
            wu_copy.wait()
            wd_copy.wait()

        @pl.when(layer == 1)
        def _():
            out_copy(NSEG - 2).start()
            out_copy(NSEG - 1).start()

        idx, ys, sub = ffn()

        @pl.when(layer == 1)
        def _():
            for s in range(NSEG):
                out_copy(s).wait()

        patch(idx, ys, sub)

        @pl.when(layer == 0)
        def _():
            for ii in idx:
                @pl.when(ii < L)
                def _():
                    b = (ii >> 4) << 4
                    ln_a(XN, b, b, 16)

        @pl.when(layer == 1)
        def _():
            bs = [pl.multiple_of((ii >> 4) << 4, 16) for ii in idx]
            cps = [pltpu.make_async_copy(X.at[pl.ds(b, 16), :], out_hbm.at[0, pl.ds(b, 16), :], sem_o.at[j])
                   for j, b in enumerate(bs)]
            cps[0].start()

            @pl.when(bs[0] != bs[1])
            def _():
                cps[1].start()
                cps[1].wait()

            cps[0].wait()

        return carry

    for c in range(L // 128):
        x0_copy(c).wait()
        XN[c * 128:(c + 1) * 128, :] = _ln(X[c * 128:(c + 1) * 128, :].astype(f32)).astype(bf16)
    for cp in w_copies(0):
        cp.wait()
    x0_copy(4).wait()

    lax.fori_loop(0, 2, layer_body, 0)


def _pk(*shape):
    return pltpu.VMEM((*shape[:-2], shape[-2] // 2, shape[-1]), u32)


@jax.jit
def pallas_interleave_layers__memory_aug_infini_attn__moe_arch_mod__prompt_kernel(
    A_x: jax.Array,
    A_wq: jax.Array,
    A_wk: jax.Array,
    A_wv: jax.Array,
    A_wo: jax.Array,
    A_beta: jax.Array,
    B_x: jax.Array,
    B_w_r: jax.Array,
    B_w_gate: jax.Array,
    B_w_up: jax.Array,
    B_w_down: jax.Array,
):
    del B_x
    any_spec = pl.BlockSpec(memory_space=pl.ANY)
    vmem_spec = pl.BlockSpec(memory_space=pltpu.VMEM)
    scratch = [
        _pk(2 * XBO, D),
        _pk(2 * L, D),
        _pk(2 * CH, D),
        _pk(G, D, 384),
        _pk(D, D),
        _pk(D, F),
        _pk(D, F),
        _pk(F, D),
        _pk(2 * L, 256),
        _pk(2 * L, 256),
        _pk(2 * L, 256),
        _pk(2 * 128, L),
        _pk(2 * G * L, 256),
        _pk(2 * G * MR, L),
        _pk(2 * G * L + 16, 256),
        _pk(MR, 256),
        _pk(QB, 512), _pk(2 * QB, 512), _pk(3 * QB, 512), _pk(4 * QB, 512),
        _pk(2 * CH + L, D),
        _pk(2 * QB, 256), _pk(2 * QB, 256), _pk(2 * QB, 256), _pk(2 * QB, 256),
        _pk(SB, D), _pk(SB, D),
        pltpu.VMEM((2 * SB, 128), f32), pltpu.VMEM((2 * SB, 128), f32),
        pltpu.VMEM((QB, 512), f32), pltpu.VMEM((2 * QB, 512), f32),
        pltpu.VMEM((3 * QB, 512), f32), pltpu.VMEM((4 * QB, 512), f32),
        pltpu.VMEM((G, MR, 128), f32),
        pltpu.VMEM((16, 128), i32),
        pltpu.VMEM((H, 128), f32),
        pltpu.VMEM((128, 128), f32),
        pltpu.VMEM((MR, 128), f32),
        pltpu.VMEM((8, D), f32),
        pltpu.SMEM((8,), i32),
        pltpu.SemaphoreType.DMA((NSEG + 5,)),
        pltpu.SemaphoreType.DMA((3 * G + 1,)),
        pltpu.SemaphoreType.DMA((3,)),
        pltpu.SemaphoreType.DMA((NSEG,)),
    ]
    return pl.pallas_call(
        _kernel,
        out_shape=jax.ShapeDtypeStruct((1, S, D), bf16),
        in_specs=[any_spec, any_spec, any_spec, any_spec, any_spec, vmem_spec, vmem_spec,
                  any_spec, any_spec, any_spec],
        out_specs=any_spec,
        scratch_shapes=scratch,
        compiler_params=pltpu.CompilerParams(vmem_limit_bytes=100 * 2 ** 20),
    )(A_x, A_wq, A_wk, A_wv, A_wo, A_beta.reshape(1, H), B_w_r.reshape(1, D), B_w_gate, B_w_up, B_w_down)
```

```python
import functools
import math

import jax
import jax.numpy as jnp
from jax import lax
import jax.experimental.pallas as pl
import jax.experimental.pallas.tpu as pltpu

S = 2048
D = 1024
H = 32
DH = 32
NSEG = 4
L = S // NSEG
F = 3584
G = 8
HG = 4
QB = 128
NQB = L // QB
MR = 144
CH = L // G
U = 2
SB = 32
PD = 16
E3N = 42
PDL = 16
PVP = {0: 3, 12: 0, 28: 1, 50: 2}
PE = 4
XBO = S + CH
EPS = 1e-5
LOG2E = math.log2(math.e)
QSCALE = (DH ** -0.5) * LOG2E
NEG = -1e9 * LOG2E
IMIN = -2 ** 31

f32 = jnp.float32
bf16 = jnp.bfloat16
i32 = jnp.int32
u32 = jnp.uint32

NT = (((1,), (1,)), ((), ()))


def _rbf(x):
    return x.astype(bf16).astype(f32)


def _recip(x):
    r = pl.reciprocal(x, approx=True)
    return r * (2.0 - x * r)


def _rstd(v):
    a = _rbf(_rbf(v) + EPS)
    y = lax.rsqrt(a)
    sd = _rbf(a * y)
    return y * (2.0 - sd * y)


def _ln(x):
    m = jnp.sum(x, axis=1, keepdims=True) * (1.0 / D)
    mb = _rbf(m)
    c = x - mb
    e = m - mb
    return c * _rstd(jnp.maximum(jnp.sum(c * c, axis=1, keepdims=True) * (1.0 / D) - e * e, 0.0))


def _stats(xs):
    p = jnp.broadcast_to(xs[0][:, 0:1], xs[0].shape)
    s = q = None
    for xc in xs:
        d = xc - p
        s = d if s is None else s + d
        q = d * d if q is None else q + d * d
    sm = jnp.sum(s, axis=1, keepdims=True) * (1.0 / D)
    v = jnp.sum(q, axis=1, keepdims=True) * (1.0 / D) - sm * sm
    return _rbf(p + sm), _rstd(v)


def _phi(t):
    return jnp.where(t > 0, t + 1.0, jnp.exp(t))


def _sigmoid(t):
    return 1.0 / (1.0 + jnp.exp(-t))


def _dot(a, b):
    return jnp.dot(a, b, preferred_element_type=f32)


def _dot_nt(a, b):
    return lax.dot_general(a, b, NT, preferred_element_type=f32)


def _ds(start, size, mult):
    if isinstance(start, int):
        return pl.ds(start, size)
    return pl.ds(pl.multiple_of(start, mult), size)


def _colred(p, op, nacc=2):
    n = p.shape[0]
    parts = [p[j * 8:(j + 1) * 8] for j in range(n // 8)]
    acc = parts[:nacc]
    for j in range(nacc, len(parts)):
        acc[j % nacc] = op(acc[j % nacc], parts[j])
    r = acc[0]
    for a in acc[1:]:
        r = op(r, a)
    return r


def _kernel(x_hbm, wq_hbm, wk_hbm, wv_hbm, wo_hbm, beta_ref, wr_ref, wg_hbm, wu_hbm, wd_hbm,
            out_hbm,
            X, XN, LS, W3, WO, WG, WU, WD,
            KB, QS, PQ, VT, PKS, VTS, OB, MEMB, PB0, PB1, PB2, PB3, YB, OS0, OS1, OS2, OS3, XS0, XS1, ST0, ST1,
            SC0, SC1, SC2, SC3, MEM, TOP, GATE, MASK, MMASK, WR, ZS,
            sem_x, sem_w, sem_f, sem_o):
    X, XN, LS, W3, WO, WG, WU, WD, KB, QS, PQ, VT, PKS, VTS, OB, MEMB, YB = [
        r.bitcast(bf16) for r in
        (X, XN, LS, W3, WO, WG, WU, WD, KB, QS, PQ, VT, PKS, VTS, OB, MEMB, YB)]
    PB = [r.bitcast(bf16) for r in (PB0, PB1, PB2, PB3)]
    OS = [r.bitcast(bf16) for r in (OS0, OS1, OS2, OS3)]
    XS = [r.bitcast(bf16) for r in (XS0, XS1)]
    ST = (ST0, ST1)
    SC = (SC0, SC1, SC2, SC3)

    def x0_copy(c):
        return pltpu.make_async_copy(x_hbm.at[0, pl.ds(c * 128, 128), :], X.at[pl.ds(c * 128, 128), :],
                                     sem_x.at[NSEG + c])

    def x_copy(s):
        r0 = s * L + (128 if s == 1 else 0)
        n = (s + 1) * L - r0
        return pltpu.make_async_copy(x_hbm.at[0, pl.ds(r0, n), :], X.at[pl.ds(r0, n), :], sem_x.at[s])

    def w_copies(g):
        col = pl.multiple_of(g * 128, 128)
        return [pltpu.make_async_copy(w.at[:, pl.ds(col, 128)], W3.at[g, :, pl.ds(j * 128, 128)],
                                      sem_w.at[3 * g + j])
                for j, w in enumerate((wk_hbm, wq_hbm, wv_hbm))]

    wo_copy = pltpu.make_async_copy(wo_hbm, WO, sem_w.at[3 * G])
    wg_copy = pltpu.make_async_copy(wg_hbm, WG, sem_f.at[0])
    wu_copy = pltpu.make_async_copy(wu_hbm, WU, sem_f.at[1])
    wd_copy = pltpu.make_async_copy(wd_hbm, WD, sem_f.at[2])

    def out_copy(s):
        base = pl.multiple_of(s * L, L)
        return pltpu.make_async_copy(X.at[pl.ds(base, L), :], out_hbm.at[0, pl.ds(base, L), :], sem_o.at[s])

    x0_copy(0).start()
    for cp in w_copies(0):
        cp.start()
    for c in range(1, 5):
        x0_copy(c).start()
    for g in range(1, 1 + U):
        for cp in w_copies(g):
            cp.start()
    x_copy(1).start()

    row = lax.broadcasted_iota(i32, (128, 128), 0)
    col = lax.broadcasted_iota(i32, (128, 128), 1)
    MASK[...] = jnp.where(row > col, NEG, 0.0).astype(f32)
    r144 = lax.broadcasted_iota(i32, (MR, 128), 0)
    c144 = lax.broadcasted_iota(i32, (MR, 128), 1)
    head_of_row = jnp.where(r144 < 128, r144 >> 5, r144 - 128)
    MMASK[...] = jnp.where(head_of_row == (c144 >> 5), 1.0, 0.0).astype(f32)
    for t in range(2 * G):
        VTS[t * MR + 128:(t + 1) * MR, :] = jnp.ones((MR - 128, L), bf16)
    for j in range(8):
        ZS[j] = 0
    X[S:S + CH, :] = jnp.zeros((CH, D), bf16)
    for r in OS:
        r[:, 0:128] = jnp.zeros((2 * QB, 128), bf16)
    OB[2 * G * L:2 * G * L + 16, 0:128] = jnp.zeros((16, 128), bf16)
    YB[CH:2 * CH, :] = jnp.zeros((CH, D), bf16)
    gsig = _rbf(_sigmoid(beta_ref[...].astype(f32).reshape(1, H)))
    r32 = lax.broadcasted_iota(i32, (H, H), 0)
    c32 = lax.broadcasted_iota(i32, (H, H), 1)
    gcol = jnp.sum(jnp.where(r32 == c32, jnp.broadcast_to(gsig, (H, H)), 0.0), axis=1, keepdims=True)
    GATE[...] = jnp.broadcast_to(gcol, (H, 128))
    WR[...] = jnp.broadcast_to(wr_ref[...].astype(f32).reshape(1, D), (8, D))

    lane128 = lax.broadcasted_iota(i32, (QB // 2, 128), 1) >> 5

    def gated(x, gate, slots=None):
        if gate is None and not slots:
            return x
        xu = pltpu.bitcast(x, u32)
        slots = dict(slots or {})
        if gate is not None:
            for t in range(4):
                slots[(t, 0)] = gate if (t, 0) not in slots else slots[(t, 0)] | gate
        rows = []
        for b in range(xu.shape[0] // 8):
            blk = xu[b * 8:(b + 1) * 8]
            if any(k[1] == b for k in slots):
                blk = jnp.concatenate(
                    [blk[:, t * 128:(t + 1) * 128] | slots[(t, b)] if (t, b) in slots else blk[:, t * 128:(t + 1) * 128]
                     for t in range(xu.shape[1] // 128)], axis=1)
            rows.append(blk)
        return pltpu.bitcast(jnp.concatenate(rows, axis=0), bf16)

    def spread(gates, nb, first=0):
        return {(4 * (i // nb) + i % 4, i % nb): gt for i, gt in enumerate(gates, first)}

    def done(*vals):
        acc = None
        for v in vals:
            w = pltpu.bitcast(v, u32)
            for r in range(0, w.shape[0], 8):
                for c in range(0, w.shape[1], 128):
                    t = w[r:r + 8, c:c + 128]
                    acc = t if acc is None else acc | t
        return acc & jnp.full((8, 128), ZS[3], i32).astype(u32)

    def after(x, gate):
        if gate is None:
            return x
        xu = pltpu.bitcast(x, u32)
        return pltpu.bitcast(xu | jnp.tile(gate, (xu.shape[0] // 8, xu.shape[1] // 128)), bf16)

    def proj_part(kind, c, par, g, slot, gate=None, slots=None):
        rows = slice(c * 128, (c + 1) * 128)
        srows = slice(slot * L + c * 128, slot * L + (c + 1) * 128)
        item = par * G + g
        j = 'kqv'.index(kind)
        x = XN[_ds(par * L + c * 128 + ZS[j], 128, 128), :]
        x = gated(x, gate, slots)
        r = _dot(x, W3[g, :, j * 128:(j + 1) * 128])
        if kind == 'v':
            vt = r.astype(bf16).T
            VT[slot * 128:(slot + 1) * 128, rows] = vt
            VTS[_ds(item * MR, 128, 16), rows] = vt
            return [jnp.abs(r[t * 8:(t + 1) * 8]) for t in range(16)] + [done(vt)]
        ph = _phi(r)
        if kind == 'k':
            KB[srows, 0:128] = r.astype(bf16)
            PKS[_ds(item * L + c * 128, 128, 128), 0:128] = ph.astype(bf16)
        else:
            QS[srows, 0:128] = (r * QSCALE).astype(bf16)
            PQ[srows, 0:128] = ph.astype(bf16)
        return [ph[t * 8:(t + 1) * 8] for t in range(16)]

    def mem_update(par, g):
        prev = (1 - par) * G + g
        m = MEM[g] + _dot(VTS[_ds(prev * MR, MR, 16), :], PKS[_ds(prev * L, L, L), 0:128])
        MEM[g] = m
        MEMB[:, 0:128] = (m * MMASK[...]).astype(bf16)

    def qk(i, slot, gate=None):
        n = QB * (i + 1)
        qi = pltpu.bitcast(QS[slot * L + i * QB:slot * L + (i + 1) * QB, 0:128], u32)
        qm = jnp.concatenate(
            [pltpu.bitcast(jnp.where(lane128 == h, qi, jnp.uint32(0)), bf16) for h in range(HG)], axis=0)
        kb = KB[slot * L:slot * L + n, 0:128]
        if gate is not None:
            kb = jnp.concatenate([after(kb[0:16], gate), kb[16:]], axis=0)
        st = _dot_nt(kb, qm)
        ms = []
        for h in range(HG):
            sh = st[:, h * QB:(h + 1) * QB]
            sd = sh[n - QB:, :] + MASK[...]
            sh = sd if i == 0 else jnp.concatenate([sh[:n - QB, :], sd], axis=0)
            SC[i][:, h * QB:(h + 1) * QB] = sh
            ms.append(jnp.max(_colred(sh, jnp.maximum), axis=0, keepdims=True))
        return ms + [st[t:t + 8, 0:QB] for t in range(0, n, 16)]

    def expo(i, h, ms, hist, rel, PD=PD):
        n = QB * (i + 1)
        z = ZS[0]
        sc = SC[i][_ds(z, n, 8), h * QB:(h + 1) * QB]
        m = jnp.broadcast_to(ms[h], (8, QB))
        ps = []
        acc = [None, None]
        for k in range(n // 8):
            if k % PE == 0:
                pace = rel[k // PE] if rel is not None else (hist[-PD] if len(hist) >= PD else None)
                mk = m if pace is None else m + jnp.minimum(pace, 0.0)
            pk = jnp.exp2(sc[k * 8:(k + 1) * 8] - mk)
            acc[k % 2] = pk if acc[k % 2] is None else acc[k % 2] + pk
            hist.append(acc[k % 2])
            ps.append(pk)
        PB[i][:, h * QB:(h + 1) * QB] = jnp.concatenate(ps, axis=0).astype(bf16)
        return acc[0] + acc[1]

    def pv(i, ls, use_mem, par, g, slot):
        n = QB * (i + 1)
        if use_mem:
            mrd = _dot_nt(MEMB[:, 0:128], PQ[slot * L + i * QB:slot * L + (i + 1) * QB, 0:128])
        outs = []
        z = ZS[0]
        for h in range(HG):
            o = _dot(VT[slot * 128 + h * DH:slot * 128 + (h + 1) * DH, 0:n], PB[i][_ds(z, n, 16), h * QB:(h + 1) * QB])
            gt = GATE[pl.ds(g * HG + h, 1), :]
            o = o * ((1.0 - gt) * _recip(jnp.sum(ls[h], axis=0, keepdims=True)))
            if use_mem:
                num = mrd[h * DH:(h + 1) * DH, :]
                den = mrd[128 + h:129 + h, :] + 1e-6
                o = num * (gt * _recip(den)) + o
            outs.append(o)
        ot = jnp.concatenate(outs, axis=0)
        ot = ot.astype(bf16).T
        OS[i][slot * QB:(slot + 1) * QB, 0:128] = ot
        return done(ot)

    def flush(par, g):
        XN[_ds((1 - par) * L + g * CH, 2 * CH, 2 * CH), :] = LS[...]
        g1 = done(XN[_ds(ZS[4], 16, 16), 0:128])
        prev = (par * G + g + 2 * G - 2) % (2 * G)
        for u in range(2):
            for i in range(NQB):
                OB[_ds((prev + u) * L + i * QB, QB, QB), 0:128] = OS[i][u * QB:(u + 1) * QB, 0:128]
        return g1, done(OB[_ds(2 * G * L + ZS[4], 16, 16), 0:128])

    def wo_part(j, par, r0, y0, n, gate=None, live=None, slots=None):
        o = [OB[_ds((par * G + g) * L + r0 + ZS[j], n, 16), 0:128] for g in range(G if live is None else G - 2)]
        if live is not None:
            o += [OS[r0 // QB][_ds(u * QB + r0 % QB + ZS[j], n, 16), 0:128] for u in range(2)]
        o = jnp.concatenate(o, axis=1)
        y = _dot(gated(o, gate, slots), WO[:, j * 128:(j + 1) * 128])
        YB[y0:y0 + n, j * 128:(j + 1) * 128] = y.astype(bf16)
        return [y[t:t + 8] for t in range(0, n, 16)]

    def chunks(ref, rows, rel, skip=0):
        out = []
        for c in range(D // 128):
            gate = None if (rel is None or c < skip) else rel[c * len(rel) // 8]
            out.append(after(ref[rows, c * 128:(c + 1) * 128], gate).astype(f32))
        return out

    def post1(row0, y0, n, xs, rel=None, park=False):
        x = chunks(X, _ds(row0, n, 16), rel, 1)
        y = chunks(YB, slice(y0, y0 + n), rel, 1)
        x1 = [(a + b).astype(bf16) for a, b in zip(x, y)]
        XS[xs][...] = jnp.concatenate(x1, axis=1)
        st = _stats([a.astype(f32) for a in x1])
        if park:
            st = (st[0], jnp.broadcast_to(st[1], (n, 128)))
            ST[xs][0:n, :] = st[0]
            ST[xs][n:2 * n, :] = st[1]
        else:
            st = (st[0] + jnp.minimum(st[1], 0.0), st[1])
        return st, [done(a) for a in x1]

    def post2(row0, n, xs, st, cs, rel=None, r=None):
        mb, rs = st
        out = []
        for i, c in enumerate(cs):
            cols = slice(c * 128, (c + 1) * 128)
            x1 = after(XS[xs][_ds(ZS[5], n, 16), cols], None if rel is None else rel[i]).astype(f32)
            xb16 = ((x1 - mb) * rs).astype(bf16)
            xb = xb16.astype(f32)
            X[_ds(XBO + row0, n, 16), cols] = xb16
            xo = (x1 + xb).astype(bf16)
            X[_ds(row0, n, 16), cols] = xo
            out.append(done(xo))
            t = xb * WR[0:1, cols]
            r = t if r is None else r + t
        return r, out

    def post3(row0, n, r, fresh=None):
        r = _rbf(jnp.sum(r, axis=1, keepdims=True))
        bits = pltpu.bitcast(jnp.broadcast_to(r, (n, 128)), i32)
        key = bits ^ ((bits >> 31) & 0x7FFF0000)
        key = key | (S - 1 - row0 - lax.broadcasted_iota(i32, (n, 128), 0))
        t1 = TOP[0:8, :]
        t2 = TOP[8:16, :]
        for j in range(n // 8):
            kj = key[j * 8:(j + 1) * 8]
            t2 = jnp.maximum(t2, jnp.minimum(t1, kj))
            t1 = jnp.maximum(t1, kj)
        if fresh is not None:
            t1 = jnp.where(fresh, IMIN, t1)
            t2 = jnp.where(fresh, IMIN, t2)
        TOP[0:8, :] = t1
        TOP[8:16, :] = t2
        return done(t2)

    cnt = [0]

    def post_rows(row0, y0, n, fresh=None, rel=None):
        cnt[0] += 1
        xs = cnt[0] % 2
        r, xo = post2(row0, n, xs, post1(row0, y0, n, xs, None if rel is None else [rel])[0], range(8))
        return functools.reduce(lambda a, b: a | b, xo, post3(row0, n, r, fresh))

    def ln_a(dst_ref, src, dst, n, rel=None, rel2=None):
        mb, rs = _stats(chunks(X, _ds(src, n, 16), rel, 1))
        mb = mb + jnp.minimum(rs, 0.0)
        y = [((a - mb) * rs).astype(bf16) for a in chunks(X, _ds(src + ZS[5], n, 16), rel2)]
        dst_ref[_ds(dst, n, 16), :] = jnp.concatenate(y, axis=1)
        return [done(a) for a in y]

    def group_iter(s, g, slot, first_seg, nxt, tail=False):
        par = s % 2
        r0 = g * CH
        mem = not first_seg
        last = nxt is None
        if last:
            P = lambda kind, c, *pins, **kw: None
        else:
            def P(kind, c, *pins, extra=(), slots=None):
                gate = None
                if pins:
                    v = pins[0]
                    for w in pins[1:]:
                        v = v + w
                    gate = pltpu.bitcast(jnp.minimum(v, 0.0), u32)
                for e in extra:
                    if e is not None:
                        gate = e if gate is None else gate | e
                return proj_part(kind, c, nxt[0], nxt[1], 1 - slot, gate, slots)
        if mem:
            row0 = (s - 1) * L + r0
            if isinstance(row0, int):
                prow, fresh = row0 - CH, None
            else:
                fresh = row0 == 0
                prow = jnp.where(fresh, S, row0 - CH)
        fg = flush(par, g) if slot == 0 else (None, None)
        lsrc = ((s + 1) * L + r0 + 2 * CH) % S

        dn = lambda vs: [done(v) for v in vs]

        def LN(t, rel, rel2):
            return [] if tail else ln_a(LS, lsrc + t, slot * CH + t, SB, None if rel is None else dn(rel), dn(rel2))

        if mem:
            mem_update(par, g)
        hist = []

        def E(i, h, ms, rel, off=0):
            return expo(i, h, ms, hist, None if rel is None else rel[off:], PDL if last else PD)

        if last:
            zf = lambda v: pltpu.bitcast(done(v), f32)
            m3 = qk(3, slot)
            m2 = qk(2, slot)
            m0 = qk(0, slot)
            m1 = qk(1, slot)
            sm = m2[HG:] + m0[HG:] + m1[HG:]
            l3 = [E(3, h, m3, [zf(sm[(16 * h + k) * E3N // 64]) for k in range(16)]) for h in range(HG)]
            base = s * L
            yb = 2 * CH
            wins = [(None, CH)] + [(b * QB + t, CH) for b in (3, 0, 1, 2) for t in (0, CH)]
            rows = [(prow, (1 - slot) * CH), (row0, slot * CH)] + [(base + r, yb + r) for r, _ in wins[1:]]
            stages = []
            for r, y in rows[:9]:
                stages += [(1, r, y, 0), (1, r + SB, y + SB, 1), (2, r, y, 0), (2, r + SB, y + SB, 1)]
            gates, slots, st, smp, ls = {}, {}, {}, [], [[], [], [], l3]

            def pin(gate, v):
                z = pltpu.bitcast(jnp.minimum(v, 0.0), u32)
                return z if gate is None else gate | z

            def due(p, e, first=4):
                if p < G * len(wins):
                    slots[p] = spread(e, 4, first) if wins[p // G][1] == CH else {(4 + i, i % 2): v for i, v in enumerate(e)}

            def part(p):
                ra0, n = wins[p // G]
                if ra0 is None:
                    res = wo_part(p % G, 1 - par, r0, slot * CH, CH, gates.get(p), None, slots.get(p))
                else:
                    res = wo_part(p % G, par, ra0, yb + ra0, n, gates.get(p), slot, slots.get(p))
                return [v for v in dn(res) for _ in range(CH // n)]

            for q, sg in enumerate(stages):
                p = 2 * q
                ra = part(p)
                if sg is not None and sg[0] == 2:
                    r, e = post2(sg[1], SB, sg[3], st[sg[3]], range(4), ra)
                    due(p + 2, e)
                rb = part(p + 1)
                if sg is not None and sg[0] == 1:
                    st[sg[3]], e = post1(sg[1], sg[2], SB, sg[3], ra + rb)
                    due(p + 2, e[:4])
                    due(p + 3, e[4:], 0)
                    gates[p + 5] = done(st[sg[3]][0]) if p + 5 not in gates else gates[p + 5] | done(st[sg[3]][0])
                elif sg is not None:
                    r, e = post2(sg[1], SB, sg[3], st[sg[3]], range(4, 8), rb, r)
                    due(p + 3, e)
                    gates[p + 8] = post3(sg[1], SB, r)
                smp += ra + rb
                for i, e0 in ((0, 0), (1, 8), (2, 24)):
                    w = 2 * (i + 1)
                    if e0 < p + 2 <= e0 + HG * w and (p + 2 - e0) % w == 0:
                        ls[i].append(E(i, len(ls[i]), (m0, m1, m2)[i], [pltpu.bitcast(v, f32) for v in smp[-4 * w::2]]))
                        gates[p + 4] = pin(gates.get(p + 4), ls[i][-1])
                if p in PVP:
                    pv(PVP[p], ls[PVP[p]], mem, par, g, slot)
            for t in (0, SB):
                post_rows(rows[9][0] + t, rows[9][1] + t, SB)
            return

        m3 = qk(3, slot, fg[0])
        lg0 = LN(0, m3[HG:HG + 8] if slot else None, m3[HG + 20:HG + 28])
        lg1 = LN(SB, m3[HG + 8:HG + 16], m3[HG + 28:HG + 32])
        ra = P('k', 0, slots=spread(lg0, 8, 8))
        l3 = [E(3, 0, m3, None)]
        rb = P('k', 1, slots=spread(lg1, 8))
        l3.append(E(3, 1, m3, ra))
        ra = P('k', 2, l3[0])
        m2 = qk(2, slot)
        l3.append(E(3, 2, m3, rb))
        two = lambda gs: {k: v for i, gt in enumerate(gs) for k, v in spread([gt], 8, 2 * i).items()}
        if mem:
            sa, da = post1(prow, (1 - slot) * CH, SB, 0, dn(m2[HG::3]), True)
        rb = P('k', 3, l3[1], extra=[fg[1]], slots=two(da) if mem else None)
        m0 = qk(0, slot)
        m1 = qk(1, slot)
        l3.append(E(3, 3, m3, ra))
        if mem:
            sb, db = post1(prow + SB, (1 - slot) * CH + SB, SB, 1, dn((m0[HG:] + m1[HG:])[::3]), True)
        ra = P('q', 3, l3[2], extra=[done(*sa)] if mem else [], slots=two(db) if mem else None)
        l2 = [E(2, 0, m2, rb)]
        l0 = [E(0, 0, m0, rb, 12)]
        rb = P('v', 0, l3[3])
        o3 = pv(3, l3, mem, par, g, slot)
        vd = [rb[16]]
        for h in range(1, HG):
            l2.append(E(2, h, m2, ra))
            l0.append(E(0, h, m0, ra, 12))
            ra, rb = rb, P('v', h, l2[h - 1], l0[h - 1], extra=[o3, vd[0]] if h == 3 else [done(*sb)] if h == 1 and mem else [])
            vd.append(rb[16])
        l1 = [E(1, h, m1, ra, 8 * h) for h in range(2)]
        ra = P('q', 2, l2[3], l0[3], extra=[vd[1]])
        o2 = pv(2, l2, mem, par, g, slot)
        o0 = pv(0, l0, mem, par, g, slot)
        l1 += [E(1, h, m1, rb, 8 * (h - 2)) for h in range(2, 4)]
        ra = P('q', 1, *l1, extra=[vd[2]])
        o1 = pv(1, l1, mem, par, g, slot)
        if not mem:
            P('q', 0, extra=[vd[3]])
            return
        P('q', 0, extra=[vd[3]])
        gates = {1: o2 | o0, 4: o1}
        slots = {}
        sa, sb = [(ST[i][_ds(ZS[5], SB, 8), :], ST[i][_ds(SB + ZS[5], SB, 8), :]) for i in range(2)]
        r = None
        for j in range(G):
            res = wo_part(j, 1 - par, r0, slot * CH, CH, gates.get(j), None, slots.get(j))
            if j < 4:
                row = prow + SB * (j // 2)
                r, e = post2(row, SB, j // 2, sb if j // 2 else sa, range(4 * (j % 2), 4 * (j % 2) + 4), dn(res), r)
                slots[j + 2] = spread(e, 4, 4)
                if j == 1:
                    gates[6] = post3(row, SB, r, fresh)
                    r = None
                if j == 3:
                    t = post3(row, SB, r, fresh)
                    slots[7] = {(4 + i, 0): t for i in range(4)}

    def ffn():
        t = TOP[...]
        k1 = jnp.max(t, axis=0, keepdims=True)
        k2 = jnp.max(jnp.where(t == k1, IMIN, t), axis=0, keepdims=True)
        sub = lax.broadcasted_iota(i32, (16, D), 0)
        idx, blks, sgs = [], [], []
        for kk in (k1, k2):
            ii = jnp.clip(S - 1 - (kk[0, 0] & 0xFFFF), 0, S - 1)
            hi = kk & (-65536)
            rv = pltpu.bitcast(hi ^ ((hi >> 31) & 0x7FFF0000), f32)
            sgs.append(_rbf(_sigmoid(rv))[:, 0:1])
            idx.append(ii)
            blks.append(X[pl.ds(pl.multiple_of(XBO + ((ii >> 4) << 4), 16), 16), :])
        xs = jnp.concatenate(blks, axis=0)
        gt = _rbf(_dot(xs, WG[...]))
        up = _rbf(_dot(xs, WU[...]))
        hh = (_rbf(gt * _sigmoid(gt)) * up).astype(bf16)
        nk = 4
        kc = F // nk
        y = _dot(hh[:, 0:kc], WD[0:kc, :])
        for j in range(1, nk):
            y = y + _dot(hh[:, j * kc:(j + 1) * kc], WD[j * kc:(j + 1) * kc, :])
        y = _rbf(y)
        return idx, [_rbf(y[j * 16:(j + 1) * 16, :] * sgs[j]) for j in range(2)], sub

    def patch(idx, ys, sub):
        for ii, yj in zip(idx, ys):
            b = pl.multiple_of((ii >> 4) << 4, 16)
            blk = X[pl.ds(b, 16), :].astype(f32)
            X[pl.ds(b, 16), :] = jnp.where(sub == (ii & 15), blk + yj, blk).astype(bf16)

    def layer_body(layer, carry):
        MEM[...] = jnp.zeros(MEM.shape, f32)
        TOP[...] = jnp.full(TOP.shape, IMIN, i32)
        lg = [functools.reduce(lambda a, b: a | b, ln_a(LS, L + t, t, CH)) for t in (0, CH)]
        for kind in 'vkq':
            for c in range(4):
                proj_part(kind, c, 0, 0, 0, lg[c // 2] if (kind == 'k' and c % 2 == 1) else None)

        @pl.when(layer == 0)
        def _():
            x_copy(1).wait()

        def body_a(j, c):
            @pl.when(layer == 0)
            def _():
                for u in range(U):
                    g = j * U + u + 1

                    @pl.when(g < G)
                    def _():
                        for cp in w_copies(g):
                            cp.wait()

                    @pl.when(g + U < G)
                    def _():
                        for cp in w_copies(g + U):
                            cp.start()

                @pl.when(j == 1)
                def _():
                    wo_copy.start()
                    x_copy(2).start()
                    x_copy(3).start()

                @pl.when(j == G // U - 1)
                def _():
                    x_copy(2).wait()

            for u in range(U):
                g = j * U + u
                if u < U - 1:
                    nxt = (0, g + 1)
                else:
                    nxt = (jnp.where(j == G // U - 1, 1, 0), (g + 1) % G)
                group_iter(0, g, u % 2, True, nxt)
            return c

        lax.fori_loop(0, G // U, body_a, 0)

        @pl.when(layer == 0)
        def _():
            wo_copy.wait()
            x_copy(3).wait()
            wg_copy.start()
            wu_copy.start()
            wd_copy.start()

        def body_b(it, c):
            s = 1 + it // (G // U)
            j = it % (G // U)
            for u in range(U):
                g = j * U + u
                if u < U - 1:
                    nxt = (s % 2, g + 1)
                else:
                    nxt = ((s + jnp.where(j == G // U - 1, 1, 0)) % 2, (g + 1) % G)
                group_iter(s, g, u % 2, False, nxt)

            @pl.when(jnp.logical_and(layer == 1, jnp.logical_and(j == 0, s >= 2)))
            def _():
                out_copy(jnp.maximum(s - 2, 0)).start()

            return c

        lax.fori_loop(0, 3 * (G // U) - 1, body_b, 0)
        s = NSEG - 1
        for g in range(G - U, G):
            group_iter(s, g, g % 2, False, (s % 2, g + 1) if g < G - 1 else None, tail=True)

        @pl.when(layer == 0)
        def _():
            wg_copy.wait()
            wu_copy.wait()
            wd_copy.wait()

        @pl.when(layer == 1)
        def _():
            out_copy(NSEG - 2).start()
            out_copy(NSEG - 1).start()

        idx, ys, sub = ffn()

        @pl.when(layer == 1)
        def _():
            for s in range(NSEG):
                out_copy(s).wait()

        patch(idx, ys, sub)

        @pl.when(layer == 0)
        def _():
            for ii in idx:
                @pl.when(ii < L)
                def _():
                    b = (ii >> 4) << 4
                    ln_a(XN, b, b, 16)

        @pl.when(layer == 1)
        def _():
            bs = [pl.multiple_of((ii >> 4) << 4, 16) for ii in idx]
            cps = [pltpu.make_async_copy(X.at[pl.ds(b, 16), :], out_hbm.at[0, pl.ds(b, 16), :], sem_o.at[j])
                   for j, b in enumerate(bs)]
            cps[0].start()

            @pl.when(bs[0] != bs[1])
            def _():
                cps[1].start()
                cps[1].wait()

            cps[0].wait()

        return carry

    for c in range(L // 128):
        x0_copy(c).wait()
        XN[c * 128:(c + 1) * 128, :] = _ln(X[c * 128:(c + 1) * 128, :].astype(f32)).astype(bf16)
    for cp in w_copies(0):
        cp.wait()
    x0_copy(4).wait()

    lax.fori_loop(0, 2, layer_body, 0)


def _pk(*shape):
    return pltpu.VMEM((*shape[:-2], shape[-2] // 2, shape[-1]), u32)


@jax.jit
def pallas_interleave_layers__memory_aug_infini_attn__moe_arch_mod__prompt_kernel(
    A_x: jax.Array,
    A_wq: jax.Array,
    A_wk: jax.Array,
    A_wv: jax.Array,
    A_wo: jax.Array,
    A_beta: jax.Array,
    B_x: jax.Array,
    B_w_r: jax.Array,
    B_w_gate: jax.Array,
    B_w_up: jax.Array,
    B_w_down: jax.Array,
):
    del B_x
    any_spec = pl.BlockSpec(memory_space=pl.ANY)
    vmem_spec = pl.BlockSpec(memory_space=pltpu.VMEM)
    scratch = [
        _pk(2 * XBO, D),
        _pk(2 * L, D),
        _pk(2 * CH, D),
        _pk(G, D, 384),
        _pk(D, D),
        _pk(D, F),
        _pk(D, F),
        _pk(F, D),
        _pk(2 * L, 256),
        _pk(2 * L, 256),
        _pk(2 * L, 256),
        _pk(2 * 128, L),
        _pk(2 * G * L, 256),
        _pk(2 * G * MR, L),
        _pk(2 * G * L + 16, 256),
        _pk(MR, 256),
        _pk(QB, 512), _pk(2 * QB, 512), _pk(3 * QB, 512), _pk(4 * QB, 512),
        _pk(2 * CH + L, D),
        _pk(2 * QB, 256), _pk(2 * QB, 256), _pk(2 * QB, 256), _pk(2 * QB, 256),
        _pk(SB, D), _pk(SB, D),
        pltpu.VMEM((2 * SB, 128), f32), pltpu.VMEM((2 * SB, 128), f32),
        pltpu.VMEM((QB, 512), f32), pltpu.VMEM((2 * QB, 512), f32),
        pltpu.VMEM((3 * QB, 512), f32), pltpu.VMEM((4 * QB, 512), f32),
        pltpu.VMEM((G, MR, 128), f32),
        pltpu.VMEM((16, 128), i32),
        pltpu.VMEM((H, 128), f32),
        pltpu.VMEM((128, 128), f32),
        pltpu.VMEM((MR, 128), f32),
        pltpu.VMEM((8, D), f32),
        pltpu.SMEM((8,), i32),
        pltpu.SemaphoreType.DMA((NSEG + 5,)),
        pltpu.SemaphoreType.DMA((3 * G + 1,)),
        pltpu.SemaphoreType.DMA((3,)),
        pltpu.SemaphoreType.DMA((NSEG,)),
    ]
    return pl.pallas_call(
        _kernel,
        out_shape=jax.ShapeDtypeStruct((1, S, D), bf16),
        in_specs=[any_spec, any_spec, any_spec, any_spec, any_spec, vmem_spec, vmem_spec,
                  any_spec, any_spec, any_spec],
        out_specs=any_spec,
        scratch_shapes=scratch,
        compiler_params=pltpu.CompilerParams(vmem_limit_bytes=100 * 2 ** 20),
    )(A_x, A_wq, A_wk, A_wv, A_wo, A_beta, B_w_r, B_w_gate, B_w_up, B_w_down)
```
